```python
import jax
import jax.numpy as jnp

def _softmax(x, axis=-1):
    return jax.nn.softmax(x, axis=axis)

def _gelu(x):
    return jax.nn.gelu(x, approximate=True)

def _silu(x):
    return jax.nn.silu(x)

def _sigmoid(x):
    return jax.nn.sigmoid(x)

def _layernorm(x, axis=-1, eps=1e-05):
    m = jnp.mean(x, axis=axis, keepdims=True)
    v = jnp.var(x, axis=axis, keepdims=True)
    return (x - m) / jnp.sqrt(v + eps)

def _scatter_add(tgt, idx, src, axis=0):
    return tgt.at[idx].add(src)

def _segment_sum(src, seg, n):
    return jax.ops.segment_sum(src, seg, n)

class _Rng:

    def __init__(self, key):
        self._k = key

    def _next(self):
        self._k, sub = jax.random.split(self._k)
        return sub

    def normal(self, shape):
        return jax.random.normal(self._next(), shape, dtype=jnp.bfloat16)

    def randint(self, lo, hi, shape):
        return jax.random.randint(self._next(), shape, lo, hi, dtype=jnp.int32)

    def uniform(self, shape, lo=0.0, hi=1.0):
        return jax.random.uniform(self._next(), shape, jnp.bfloat16, lo, hi)

    def permutation(self, n):
        return jax.random.permutation(self._next(), n)
kernel_name = 'gated_mix__softmax_full_mha__memory_aug_recurrent_mem_tr__prompt'

def setup_inputs():
    _rng = _Rng(jax.random.key(int.from_bytes(__import__("os").urandom(4), "little")))
    _w = lambda a: (lambda t: t.astype(jnp.bfloat16) if jnp.issubdtype(t.dtype, jnp.floating) else t)(jnp.asarray(a))

    def _A_setup():
        B, S, D = (1, 2048, 1024)
        return {'x': _w((lambda *s: _rng.normal(s) * 0.05)(B, S, D)), 'wqkv': _w((lambda *s: _rng.normal(s) * 0.05)(D, 3 * D)), 'wo': _w((lambda *s: _rng.normal(s) * 0.05)(D, D))}
    _A_in = _A_setup()

    def _B_setup():
        B, S, Dm = (1, 2048, 1024)
        H, Dh = (32, 128)
        M, seg = (8, 32)
        seg = min(seg, S)
        S = S // seg * seg
        return {'x': _w((lambda *s: _rng.normal(s) * 0.05)(B, S, Dm)), 'mem0': _w((lambda *s: _rng.normal(s) * 0.05)(B, M, Dm)), 'Wq': _w((lambda *s: _rng.normal(s) * 0.05)(Dm, H, Dh) * Dm ** (-0.5)), 'Wk': _w((lambda *s: _rng.normal(s) * 0.05)(Dm, H, Dh) * Dm ** (-0.5)), 'Wv': _w((lambda *s: _rng.normal(s) * 0.05)(Dm, H, Dh) * Dm ** (-0.5)), 'Wo': _w((lambda *s: _rng.normal(s) * 0.05)(H, Dh, Dm) * (H * Dh) ** (-0.5)), 'seg_len': seg}
    _B_in = _B_setup()
    return {'A_x': _A_in['x'], 'A_wqkv': _A_in['wqkv'], 'A_wo': _A_in['wo'], 'B_x': _B_in['x'], 'B_mem0': _B_in['mem0'], 'B_Wq': _B_in['Wq'], 'B_Wk': _B_in['Wk'], 'B_Wv': _B_in['Wv'], 'B_Wo': _B_in['Wo'], 'B_seg_len': _B_in['seg_len'], 'gate_w': _w((lambda *s: _rng.normal(s) * 0.05)(1024))}

def reference(A_x, A_wqkv, A_wo, B_x, B_mem0, B_Wq, B_Wk, B_Wv, B_Wo, B_seg_len, gate_w):

    def _A_ref(x, wqkv, wo):
        B, S, D = x.shape
        H = 32
        Dh = D // H
        qkv = (lambda x, *d: x.transpose(*d))((x @ wqkv).reshape(B, S, 3, H, Dh), 2, 0, 3, 1, 4)
        q, k, v = (qkv[0], qkv[1], qkv[2])
        scale = Dh ** (-0.5)
        scores = jnp.einsum('bhqd,bhkd->bhqk', q, k) * scale
        p = _softmax(scores, axis=-1)
        o = jnp.einsum('bhqk,bhkd->bhqd', p, v)
        return (lambda x, *d: x.transpose(*d))(o, 0, 2, 1, 3).reshape(B, S, D) @ wo

    def _B_ref(x, mem0, Wq, Wk, Wv, Wo, seg_len):
        B, S, Dm = x.shape
        H, Dh = (Wq.shape[1], Wq.shape[2])
        M = mem0.shape[1]
        scale = Dh ** (-0.5)
        n_seg = S // seg_len
        L = M + seg_len
        idx = jnp.arange(L)
        mask = (idx[:, None] < M) | (idx[:, None] >= idx[None, :])
        mem = mem0
        outs = []
        for s in range(n_seg):
            xs = x[:, s * seg_len:(s + 1) * seg_len, :].copy()
            h = jnp.concatenate([mem, xs], axis=1)
            q = jnp.einsum('btd,dhe->bhte', h, Wq)
            k = jnp.einsum('btd,dhe->bhte', h, Wk)
            v = jnp.einsum('btd,dhe->bhte', h, Wv)
            scores = jnp.einsum('bhqe,bhke->bhqk', q, k) * scale
            scores = jnp.where(mask[None, None], scores, -1000000000.0)
            p = _softmax(scores, axis=-1)
            o = jnp.einsum('bhqk,bhke->bhqe', p, v)
            o = jnp.einsum('bhte,hed->btd', o, Wo)
            mem = o[:, :M, :].copy()
            outs.append(o[:, M:, :])
        return jnp.concatenate(outs, axis=1)
    x = A_x
    g = _sigmoid((x * gate_w).sum(-1, keepdims=True))
    a = _A_ref(x, A_wqkv, A_wo)
    b = _B_ref(x, B_mem0, B_Wq, B_Wk, B_Wv, B_Wo, B_seg_len)
    return g * a + (1 - g) * b
```

```python
import math

import jax
import jax.numpy as jnp
import jax.experimental.pallas as pl
import jax.experimental.pallas.tpu as pltpu

BF16, F32, U32 = jnp.bfloat16, jnp.float32, jnp.uint32
LOG2E = math.log2(math.e)

S, D = 2048, 1024
HA, DA = 32, 32
HB, DB = 32, 128
MEM, SEG = 8, 32
L = MEM + SEG
NSTEP = S // SEG
QT = 128
CW = 256
HALF = S // 2


def _bf(x):
    return pltpu.bitcast(x, BF16)


def _words(x):
    return pltpu.bitcast(x.astype(BF16), U32)


def _dot(a, b):
    return jnp.dot(a, b, preferred_element_type=F32)


def _dot_nt(a, b):
    return jax.lax.dot_general(a, b, (((1,), (1,)), ((), ())), preferred_element_type=F32)


def _rows(start, n):
    return pl.ds(pl.multiple_of(start, n), n)


def _transpose8(v):
    sub = jax.lax.broadcasted_iota(U32, (8, 128), 0)
    for s in (4, 2, 1):
        keep = (sub & s) == 0
        nv = list(v)
        for i in range(8):
            if i & s == 0:
                a, b = v[i], v[i + s]
                nv[i] = jnp.where(keep, a, pltpu.roll(b, s, 0))
                nv[i + s] = jnp.where(keep, pltpu.roll(a, 8 - s, 0), b)
        v = nv
    return v


def _kernel(x_hbm, wa_hbm, woa_hbm, mem_ref, wq_hbm, wk_hbm, wv_hbm, wob_hbm, gw_ref, out_hbm,
            xs, wa, woa, wb, wob, stage, ka, qa, vt, sb0, sb1, mcar, ot, oa,
            hbuf, obuf, bbuf, gbuf, outb, in_sem, st_sem, out_sem):
    NCG = D // CW

    def x_copy():
        return pltpu.make_async_copy(x_hbm.bitcast(U32), xs, in_sem.at[0])

    def wa_copy(n):
        return pltpu.make_async_copy(
            wa_hbm.bitcast(U32).at[:, pl.ds(n * CW, CW)], wa.at[n], in_sem.at[1 + n])

    def woa_copy(n):
        return pltpu.make_async_copy(
            woa_hbm.bitcast(U32).at[:, pl.ds(n * CW, CW)], woa.at[n], in_sem.at[13 + n])

    def wob_copy():
        return pltpu.make_async_copy(wob_hbm.bitcast(U32), wob, in_sem.at[17])

    def stage_copy(w_hbm, chunk, slot):
        return pltpu.make_async_copy(
            w_hbm.bitcast(U32).at[_rows(chunk * 4096, 4096)], stage.at[slot], st_sem.at[slot])

    x_copy().start()
    for n in range(3 * NCG):
        wa_copy(n).start()
    stage_copy(wq_hbm, 0, 0).start()
    stage_copy(wq_hbm, 1, 1).start()
    for n in range(NCG):
        woa_copy(n).start()
    wob_copy().start()

    sb1[...] = jnp.zeros(sb1.shape, F32)
    mcar[...] = jnp.zeros(mcar.shape, F32)
    ot[...] = jnp.zeros(ot.shape, F32)
    oa[1] = jnp.zeros(oa.shape[1:], U32)
    bbuf[1] = jnp.zeros(bbuf.shape[1:], F32)

    x_copy().wait()
    hbuf[0:MEM, :] = mem_ref[...].astype(F32)
    hbuf[MEM:L, :] = _bf(xs[0:SEG // 2, :]).astype(F32)

    gw = gw_ref[...].astype(F32)

    def gate_body(r, carry):
        xr = _bf(xs[_rows(r * 64, 64), :]).astype(F32)
        z = jnp.sum(xr * gw, axis=-1, keepdims=True)
        gbuf[_rows(r * 128, 128), :] = jnp.broadcast_to(1.0 / (1.0 + jnp.exp(-z)), (128, 128))
        return carry

    jax.lax.fori_loop(0, S // 128, gate_body, 0)

    def relayout(slot, chunk, col):
        for g in range(16):
            w = stage[slot, g * 256:(g + 1) * 256, :].reshape(8, 2, 16, 128)
            a, b = w[:, 0], w[:, 1]
            lo = (a & U32(0xFFFF)) | (b << 16)
            hi = (a >> 16) | (b & U32(0xFFFF0000))
            rows = _rows(chunk * 128 + g * 8, 8)
            for par, t in enumerate((lo, hi)):
                for half in range(2):
                    v = _transpose8([t[i, half * 8:(half + 1) * 8, :] for i in range(8)])
                    for jj in range(8):
                        wb[2 * (half * 8 + jj) + par, rows, col * 128:(col + 1) * 128] = v[jj]

    MC = 256
    b_weights = (wq_hbm, wk_hbm, wv_hbm)
    for part in range(3):
        def proj_body(n, carry, part=part):
            slot = n % 2
            pltpu.make_async_copy(
                wa_hbm.bitcast(U32).at[:, pl.ds(0, CW)], wa.at[0],
                in_sem.at[1 + part * NCG + n]).wait()
            stage_copy(b_weights[part], n, slot).wait()
            for m in range(S // MC):
                y = _dot(_bf(xs[m * MC // 2:(m + 1) * MC // 2, :]), _bf(wa[part * NCG + n]))
                if part == 2:
                    yt = _words(y.T).reshape(CW // DA, DA // 2, MC)
                    col = (m * MC) % HALF
                    vt[(m * MC) // HALF, pl.ds(n * (CW // DA), CW // DA), :, col:col + MC] = yt
                else:
                    if part == 0:
                        y = y * (DA ** -0.5 * LOG2E)
                    yw = _words(y)
                    dst = qa if part == 0 else ka
                    for t in range(CW // 128):
                        dst[n * (CW // 128) + t, m * MC // 2:(m + 1) * MC // 2, :] = (
                            yw[:, t * 128:(t + 1) * 128])
            relayout(slot, n, part)

            @pl.when(n + 2 < NCG)
            def _():
                stage_copy(b_weights[part], n + 2, slot).start()

            if part < 2:
                @pl.when(n + 2 >= NCG)
                def _():
                    stage_copy(b_weights[part + 1], n + 2 - NCG, slot).start()
            return carry

        jax.lax.fori_loop(0, NCG, proj_body, 0)

    for n in range(NCG):
        woa_copy(n).wait()
    wob_copy().wait()

    row = jax.lax.broadcasted_iota(jnp.int32, (L, L), 0)
    col = jax.lax.broadcasted_iota(jnp.int32, (L, L), 1)
    mask_b = (row < MEM) | (row >= col)
    head_lane = jax.lax.broadcasted_iota(jnp.int32, (QT // 2, 128), 1) // DA
    sbufs = (sb0, sb1)

    def a_scores(tile, qtile, i, half):
        q = qa[tile, _rows(qtile * (QT // 2), QT // 2), :]
        q = _bf(jnp.where(head_lane == i % 4, q, U32(0)))
        k = _bf(ka[tile, half * HALF // 2:(half + 1) * HALF // 2, :])
        st = _dot_nt(k, q)
        sbufs[i % 2][half * HALF:(half + 1) * HALF, :] = st
        return st.reshape(HALF // 8, 8, 128).max(axis=0)

    def a_values(head, i, half, m):
        p = jnp.exp2(sbufs[i % 2][half * HALF:(half + 1) * HALF, :] - m)
        return _dot(_bf(vt[half, head]), p.astype(BF16)), p.reshape(HALF // 8, 8, 128).sum(axis=0)

    def a_finish(i, acc, den):
        ot[i * DA:(i + 1) * DA, :] = acc / jnp.sum(den, axis=0, keepdims=True)

    def a_transpose(qtile, tile, which):
        oa[qtile % 2, tile] = _words(ot[which * 128:(which + 1) * 128, :].T)

    def mix(qtile, cg):
        o = jnp.concatenate([_bf(oa[qtile % 2, t]) for t in range(D // 128)], axis=1)
        a = _dot(o, _bf(woa[cg]))
        rows = _rows(jnp.maximum(qtile, 0) * QT, QT)
        g = gbuf[rows, :]
        g = jnp.concatenate([g] * (CW // 128), axis=1)
        outb[cg, rows, :] = (g * a + (1.0 - g) * bbuf[qtile % 2, cg]).astype(BF16)

    def out_copy(qtile, cg):
        rows = _rows(qtile * QT, QT)
        return pltpu.make_async_copy(
            outb.at[cg, rows], out_hbm.at[rows, _rows(cg * CW, CW)], out_sem)

    def b_out(h0, h1):
        return _dot(obuf[:, h0 * DB:h1 * DB], _bf(wob[h0 * DB // 2:h1 * DB // 2, :]))

    def b_values(pair, probs):
        for e, (p, den, v) in enumerate(probs):
            hd = 2 * pair + e
            obuf[:, hd * DB:(hd + 1) * DB] = _dot(p, v) / den

    def step(s, carry):
        qtile, cg = s // 4, s % 4
        sp = jnp.maximum(s - 1, 0)
        probs = None
        m_prev = mcar[0:1, :]
        for p in range(HB // 2):
            i, half = p // 2, p % 2
            qkv = [_dot(hbuf[...], _bf(wb[2 * p + e])) for e in range(2)]
            if probs is not None:
                b_values(p - 1, probs)

            mx = a_scores(2 * cg + i // 4, qtile, i, half)
            m_run = mx if half == 0 else jnp.maximum(m_run, mx)
            ip = (i - 1) % 8
            head_prev = 8 * cg + i - 1 if i > 0 else 8 * (sp % 4) + 7
            o, den = a_values(head_prev, ip, half, m_prev)
            acc, dsum = (o, den) if half == 0 else (acc + o, dsum + den)
            if half == 1:
                a_finish(ip, acc, dsum)
                m_prev = jnp.max(m_run, axis=0, keepdims=True)
                if i == 0:
                    a_transpose((s + 7) // 4, 2 * ((s + 3) % 4) + 1, 1)
                if i == 4:
                    a_transpose(qtile, 2 * cg, 0)

            probs = []
            for e in range(2):
                q = qkv[e][:, :DB] * (DB ** -0.5 * LOG2E)
                k = qkv[e][:, DB:2 * DB].astype(BF16)
                sc = jnp.where(mask_b, _dot_nt(q, k), -1e9 * LOG2E)
                pr = jnp.exp2(sc - jnp.max(sc, axis=-1, keepdims=True))
                probs.append((pr, jnp.sum(pr, axis=-1, keepdims=True),
                              qkv[e][:, 2 * DB:].astype(BF16)))
        mcar[...] = jnp.broadcast_to(m_prev, mcar.shape)

        nxt = jnp.minimum(s + 1, NSTEP - 1)
        hbuf[MEM:L, :] = _bf(xs[_rows(nxt * (SEG // 2), SEG // 2), :]).astype(F32)
        y = b_out(0, 14)
        b_values(HB // 2 - 1, probs)
        y = y + b_out(14, 30)
        y = y + b_out(30, 32)
        hbuf[0:MEM, :] = y[0:MEM].astype(BF16).astype(F32)
        for t in range(NCG):
            bbuf[qtile % 2, t, _rows(cg * SEG, SEG), :] = y[MEM:L, t * CW:(t + 1) * CW]

        mix(qtile - 1, cg)

        @pl.when(s >= 4)
        def _():
            out_copy(qtile - 1, cg).start()
        return carry

    jax.lax.fori_loop(0, NSTEP, step, 0)

    m_last = mcar[0:1, :]
    o0, d0 = a_values(HA - 1, 7, 0, m_last)
    o1, d1 = a_values(HA - 1, 7, 1, m_last)
    a_finish(7, o0 + o1, d0 + d1)
    last = S // QT - 1
    a_transpose(last, D // 128 - 1, 1)
    for cg in range(NCG):
        mix(last, cg)
        out_copy(last, cg).start()

    def drain(t, carry):
        out_copy(t // NCG, t % NCG).wait()
        return carry

    jax.lax.fori_loop(0, (S // QT) * NCG, drain, 0)


@jax.jit
def pallas_gated_mix__softmax_full_mha__memory_aug_recurrent_mem_tr__prompt_kernel(
    A_x: jax.Array,
    A_wqkv: jax.Array,
    A_wo: jax.Array,
    B_x: jax.Array,
    B_mem0: jax.Array,
    B_Wq: jax.Array,
    B_Wk: jax.Array,
    B_Wv: jax.Array,
    B_Wo: jax.Array,
    B_seg_len: jax.Array,
    gate_w: jax.Array,
):
    del B_x, B_seg_len
    assert A_x.shape == (1, S, D) and B_mem0.shape == (1, MEM, D) and B_Wq.shape == (D, HB, DB)

    hbm = pl.BlockSpec(memory_space=pl.ANY)
    vmem = pl.BlockSpec(memory_space=pltpu.VMEM)
    out = pl.pallas_call(
        _kernel,
        out_shape=jax.ShapeDtypeStruct((S, D), BF16),
        in_specs=[hbm, hbm, hbm, vmem, hbm, hbm, hbm, hbm, vmem],
        out_specs=hbm,
        scratch_shapes=[
            pltpu.VMEM((S // 2, D), U32),
            pltpu.VMEM((3 * D // CW, D // 2, CW), U32),
            pltpu.VMEM((D // CW, D // 2, CW), U32),
            pltpu.VMEM((HB, D // 2, 3 * DB), U32),
            pltpu.VMEM((HB * DB // 2, D), U32),
            pltpu.VMEM((2, 4096, 128), U32),
            pltpu.VMEM((D // 128, S // 2, 128), U32),
            pltpu.VMEM((D // 128, S // 2, 128), U32),
            pltpu.VMEM((2, HA, DA // 2, HALF), U32),
            pltpu.VMEM((S, QT), F32),
            pltpu.VMEM((S, QT), F32),
            pltpu.VMEM((8, QT), F32),
            pltpu.VMEM((8 * DA, QT), F32),
            pltpu.VMEM((2, D // 128, QT // 2, 128), U32),
            pltpu.VMEM((L, D), F32),
            pltpu.VMEM((L, HB * DB), F32),
            pltpu.VMEM((2, D // CW, QT, CW), F32),
            pltpu.VMEM((S, 128), F32),
            pltpu.VMEM((D // CW, S, CW), BF16),
            pltpu.SemaphoreType.DMA((18,)),
            pltpu.SemaphoreType.DMA((2,)),
            pltpu.SemaphoreType.DMA(()),
        ],
        compiler_params=pltpu.CompilerParams(vmem_limit_bytes=110 * 1024 * 1024),
        name="gated_mix",
    )(
        A_x.reshape(S, D), A_wqkv, A_wo, B_mem0.reshape(MEM, D),
        B_Wq.reshape(D * HB, DB), B_Wk.reshape(D * HB, DB), B_Wv.reshape(D * HB, DB),
        B_Wo.reshape(HB * DB, D), gate_w.reshape(1, D),
    )
    return out.reshape(1, S, D)
```

```python
import math

import jax
import jax.numpy as jnp
import jax.experimental.pallas as pl
import jax.experimental.pallas.tpu as pltpu

BF16, F32, U32 = jnp.bfloat16, jnp.float32, jnp.uint32
LOG2E = math.log2(math.e)

S, D = 2048, 1024
HA, DA = 32, 32
HB, DB = 32, 128
MEM, SEG = 8, 32
L = MEM + SEG
NSTEP = S // SEG
QT = 128
KC = 512
NC = S // KC
LAG = 2
RING = 4
CW = 256
NCG = D // CW
WA0 = 3 * HB


def _bf(x):
    return pltpu.bitcast(x, BF16)


def _words(x):
    return pltpu.bitcast(x.astype(BF16), U32)


def _dot(a, b):
    return jnp.dot(a, b, preferred_element_type=F32)


def _dot_nt(a, b):
    return jax.lax.dot_general(a, b, (((1,), (1,)), ((), ())), preferred_element_type=F32)


def _recip(x):
    r = pltpu.reciprocal(x, approx=True)
    return r * (2.0 - x * r)


def _rows(start, n):
    return pl.ds(pl.multiple_of(start, n), n)


def _transpose8(v):
    sub = jax.lax.broadcasted_iota(U32, (8, 128), 0)
    for s in (4, 2, 1):
        keep = (sub & s) == 0
        nv = list(v)
        for i in range(8):
            if i & s == 0:
                a, b = v[i], v[i + s]
                nv[i] = jnp.where(keep, a, pltpu.roll(b, s, 0))
                nv[i + s] = jnp.where(keep, pltpu.roll(a, 8 - s, 0), b)
        v = nv
    return v


def _kernel(x_hbm, wa_hbm, woa_hbm, mem_ref, wq_hbm, wk_hbm, wv_hbm, wob_hbm, gw_ref, out_hbm,
            xs, wt, woa, wob, stage, ka, qa, vt, sbuf, zero, mcar, ot, oa,
            hbuf, obuf, bbuf, gbuf, outb, in_sem, st_sem, out_sem):

    def x_copy():
        return pltpu.make_async_copy(x_hbm.bitcast(U32), xs, in_sem.at[0])

    def wa_copies(n):
        return [pltpu.make_async_copy(
            wa_hbm.bitcast(U32).at[:, _rows(t * 128, 128)], wt.at[WA0 + t], in_sem.at[1 + n])
            for t in (2 * n, 2 * n + 1)]

    def woa_copy(n):
        return pltpu.make_async_copy(
            woa_hbm.bitcast(U32).at[:, pl.ds(n * CW, CW)], woa.at[n], in_sem.at[13 + n])

    def wob_copy(n):
        rows = _rows(n * (HB * DB // 8), HB * DB // 8)
        return pltpu.make_async_copy(wob_hbm.bitcast(U32).at[rows], wob.at[rows], in_sem.at[17 + n])

    def stage_copy(w_hbm, chunk, slot):
        return pltpu.make_async_copy(
            w_hbm.bitcast(U32).at[_rows(chunk * 4096, 4096)], stage.at[slot], st_sem.at[slot])

    def out_copy(qtile, cg):
        rows = _rows(qtile * QT, QT)
        return pltpu.make_async_copy(
            outb.at[cg, rows], out_hbm.at[rows, _rows(cg * CW, CW)], out_sem)

    def weights(tile, n):
        return jnp.concatenate([_bf(wt[tile + t]) for t in range(n)], axis=1)

    x_copy().start()
    for cp in wa_copies(0):
        cp.start()

    for i in range(RING - LAG, RING):
        sbuf[i][...] = jnp.zeros((S, QT), F32)
    mcar[...] = jnp.zeros(mcar.shape, F32)
    ot[...] = jnp.zeros(ot.shape, F32)
    oa[1] = jnp.zeros(oa.shape[1:], U32)
    bbuf[1] = jnp.zeros(bbuf.shape[1:], F32)
    gbuf[0:QT, :] = jnp.zeros((QT, 128), F32)
    zero[0] = 0
    zero[1] = 0
    gw = jnp.broadcast_to(gw_ref[...].astype(F32), (8, D))

    def load_segment(seg):
        xr = _bf(xs[_rows(seg * (SEG // 2), SEG // 2), :]).astype(F32)
        hbuf[MEM:L, :] = xr
        z = jnp.sum(xr.reshape(SEG // 8, 8, D) * gw, axis=-1, keepdims=True).reshape(SEG, 1)
        gbuf[_rows(QT + seg * SEG, SEG), :] = jnp.broadcast_to(
            1.0 / (1.0 + jnp.exp(-z)), (SEG, 128))

    x_copy().wait()
    stage_copy(wq_hbm, 0, 0).start()
    for cp in wa_copies(1):
        cp.start()
    stage_copy(wq_hbm, 1, 1).start()
    hbuf[0:MEM, :] = mem_ref[...].astype(F32)
    load_segment(0)

    def relayout(slot, chunk, col, g):
        w = stage[slot, g * 256:(g + 1) * 256, :].reshape(8, 2, 16, 128)
        a, b = w[:, 0], w[:, 1]
        lo = (a & U32(0xFFFF)) | (b << 16)
        hi = (a >> 16) | (b & U32(0xFFFF0000))
        rows = _rows(chunk * 128 + g * 8, 8)
        for par, t in enumerate((lo, hi)):
            for half in range(2):
                v = _transpose8([t[i, half * 8:(half + 1) * 8, :] for i in range(8)])
                for jj in range(8):
                    wt[3 * (2 * (half * 8 + jj) + par) + col, rows, :] = v[jj]

    MC = 256
    b_weights = (wq_hbm, wk_hbm, wv_hbm)
    for part in range(3):
        def proj_body(n, carry, part=part):
            slot = n % 2
            cur = part * NCG + n
            for cp in wa_copies(cur):
                cp.wait()
            stage_copy(b_weights[part], n, slot).wait()

            @pl.when(cur + 2 < 3 * NCG)
            def _():
                for cp in wa_copies(cur + 2):
                    cp.start()

            if part == 1:
                wob_copy(n).start()
            for m in range(S // MC):
                y = _dot(_bf(xs[m * MC // 2:(m + 1) * MC // 2, :]), weights(WA0 + 2 * cur, 2))
                relayout(slot, n, part, 2 * m)
                relayout(slot, n, part, 2 * m + 1)
                if part == 2:
                    yt = _words(y.T).reshape(CW // DA, DA // 2, MC)
                    col = (m * MC) % KC
                    vt[(m * MC) // KC, pl.ds(n * (CW // DA), CW // DA), :, col:col + MC] = yt
                else:
                    if part == 0:
                        y = y * (DA ** -0.5 * LOG2E)
                    yw = _words(y)
                    dst = qa if part == 0 else ka
                    for t in range(CW // 128):
                        dst[n * (CW // 128) + t, m * MC // 2:(m + 1) * MC // 2, :] = (
                            yw[:, t * 128:(t + 1) * 128])

            @pl.when(n + 2 < NCG)
            def _():
                stage_copy(b_weights[part], n + 2, slot).start()

            if part < 2:
                @pl.when(n + 2 >= NCG)
                def _():
                    stage_copy(b_weights[part + 1], n + 2 - NCG, slot).start()
            return carry

        if part == 2:
            for n in range(NCG):
                woa_copy(n).start()
        jax.lax.fori_loop(0, NCG, proj_body, 0)

    for n in range(NCG):
        woa_copy(n).wait()
        wob_copy(n).wait()

    row = jax.lax.broadcasted_iota(jnp.int32, (L, L), 0)
    col = jax.lax.broadcasted_iota(jnp.int32, (L, L), 1)
    mask_b = (row < MEM) | (row >= col)
    head_lane = jax.lax.broadcasted_iota(jnp.int32, (QT // 2, 128), 1) // DA

    def a_scores(tile, qtile, i, c):
        q = qa[tile, _rows(qtile * (QT // 2), QT // 2), :]
        q = _bf(jnp.where(head_lane == i % 4, q, U32(0)))
        mx = None
        n = KC // 4
        for r in range(c * KC, (c + 1) * KC, n):
            st = _dot_nt(_bf(ka[tile, r // 2:(r + n) // 2, :]), q)
            sbuf[i % RING][r:r + n, :] = st
            m = st.reshape(n // 8, 8, 128).max(axis=0)
            mx = m if mx is None else jnp.maximum(mx, m)
        return mx

    def a_probs(i, c, m):
        p = jnp.exp2(sbuf[i % RING][_rows(zero[1] + c * KC, KC), :] - m)
        return p.astype(BF16), p.reshape(KC // 8, 8, 128).sum(axis=0)

    def a_values(head, c, p):
        return _dot(_bf(vt[c, head]), p)

    def a_finish(i, acc, den):
        ot[i * DA:(i + 1) * DA, :] = acc * _recip(jnp.sum(den, axis=0, keepdims=True))

    def a_transpose(qtile, tile, which):
        oa[qtile % 2, tile] = _words(ot[which * 128:(which + 1) * 128, :].T)

    def mix(qtile, cg):
        o = jnp.concatenate([_bf(oa[qtile % 2, t]) for t in range(D // 128)], axis=1)
        a = _dot(o, _bf(woa[cg]))
        g = gbuf[_rows((qtile + 1) * QT, QT), :]
        g = jnp.concatenate([g] * (CW // 128), axis=1)
        outb[cg, _rows(jnp.maximum(qtile, 0) * QT, QT), :] = (
            g * a + (1.0 - g) * bbuf[qtile % 2, cg]).astype(BF16)

    def b_out(h0, h1):
        return _dot(obuf[:, h0 * DB:h1 * DB], _bf(wob[h0 * DB // 2:h1 * DB // 2, :]))

    def b_scores(q, k):
        sc = jnp.where(mask_b, _dot_nt(q, k), -1e9 * LOG2E)
        pr = jnp.exp2(sc - jnp.max(sc, axis=-1, keepdims=True))
        return pr * _recip(jnp.sum(pr, axis=-1, keepdims=True))

    def b_values(hd, pr, v):
        obuf[:, hd * DB:(hd + 1) * DB] = _dot(pr, v)

    def step(s, carry):
        qtile, cg = s // 4, s % 4
        cg_prev = (s + 3) % 4
        maxes = {i - LAG: mcar[i, 0:1, :] for i in range(LAG)}
        qk, vs, prs = {}, {}, {}
        for h in range(HB):
            i, c = h // NC, h % NC
            ip = i - LAG
            p, den = a_probs(ip, c, maxes[ip])
            dsum = den if c == 0 else dsum + den

            y = _dot(hbuf[...], weights(3 * h, 2))
            qk[h] = (y[:, :DB] * (DB ** -0.5 * LOG2E), y[:, DB:].astype(BF16))

            mx = a_scores(2 * cg + i // 4, qtile, i, c)
            m_run = mx if c == 0 else jnp.maximum(m_run, mx)

            o = a_values(8 * cg + ip if ip >= 0 else 8 * cg_prev + 8 + ip, c, p)
            acc = o if c == 0 else acc + o

            vs[h] = _dot(hbuf[...], weights(3 * h + 2, 1)).astype(BF16)
            if h >= 1:
                prs[h - 1] = b_scores(*qk.pop(h - 1))
            if h >= 3:
                b_values(h - 3, prs.pop(h - 3), vs.pop(h - 3))

            if c == NC - 1:
                a_finish(ip % 8, acc, dsum)
                maxes[i] = jnp.max(m_run, axis=0, keepdims=True)
                if ip == -1:
                    a_transpose((s + 7) // 4, 2 * cg_prev + 1, 1)
                if ip == 3:
                    a_transpose(qtile, 2 * cg, 0)
        for i in range(LAG):
            mcar[i] = jnp.broadcast_to(maxes[8 - LAG + i], (8, QT))

        load_segment(jnp.minimum(s + 1, NSTEP - 1))
        y = b_out(0, 3)
        prs[HB - 1] = b_scores(*qk.pop(HB - 1))
        b_values(HB - 3, prs.pop(HB - 3), vs.pop(HB - 3))
        y = y + b_out(3, 8)
        b_values(HB - 2, prs.pop(HB - 2), vs.pop(HB - 2))
        y = y + b_out(8, 13)
        b_values(HB - 1, prs.pop(HB - 1), vs.pop(HB - 1))
        y = y + b_out(13, 32)
        hbuf[0:MEM, :] = y[0:MEM].astype(BF16).astype(F32)
        for t in range(NCG):
            bbuf[qtile % 2, t, _rows(cg * SEG, SEG), :] = y[MEM:L, t * CW:(t + 1) * CW]

        mix(qtile - 1, cg)

        @pl.when(s >= 4)
        def _():
            out_copy(qtile - 1, cg).start()
        return carry

    jax.lax.fori_loop(0, NSTEP, step, 0)

    for i in range(LAG):
        for c in range(NC):
            p, den = a_probs(i - LAG, c, mcar[i, 0:1, :])
            o = a_values(HA - LAG + i, c, p)
            acc, dsum = (o, den) if c == 0 else (acc + o, dsum + den)
        a_finish(8 - LAG + i, acc, dsum)
    last = S // QT - 1
    a_transpose(last, D // 128 - 1, 1)
    for cg in range(NCG):
        mix(last, cg)
        out_copy(last, cg).start()

    def drain(t, carry):
        out_copy(t // NCG, t % NCG).wait()
        return carry

    jax.lax.fori_loop(0, (S // QT) * NCG, drain, 0)


@jax.jit
def pallas_gated_mix__softmax_full_mha__memory_aug_recurrent_mem_tr__prompt_kernel(
    A_x: jax.Array,
    A_wqkv: jax.Array,
    A_wo: jax.Array,
    B_x: jax.Array,
    B_mem0: jax.Array,
    B_Wq: jax.Array,
    B_Wk: jax.Array,
    B_Wv: jax.Array,
    B_Wo: jax.Array,
    B_seg_len: jax.Array,
    gate_w: jax.Array,
):
    del B_x, B_seg_len
    assert A_x.shape == (1, S, D) and B_mem0.shape == (1, MEM, D) and B_Wq.shape == (D, HB, DB)

    hbm = pl.BlockSpec(memory_space=pl.ANY)
    vmem = pl.BlockSpec(memory_space=pltpu.VMEM)
    out = pl.pallas_call(
        _kernel,
        out_shape=jax.ShapeDtypeStruct((S, D), BF16),
        in_specs=[hbm, hbm, hbm, vmem, hbm, hbm, hbm, hbm, vmem],
        out_specs=hbm,
        scratch_shapes=[
            pltpu.VMEM((S // 2, D), U32),
            pltpu.VMEM((WA0 + 3 * D // 128, D // 2, 128), U32),
            pltpu.VMEM((NCG, D // 2, CW), U32),
            pltpu.VMEM((HB * DB // 2, D), U32),
            pltpu.VMEM((2, 4096, 128), U32),
            pltpu.VMEM((D // 128, S // 2, 128), U32),
            pltpu.VMEM((D // 128 + 1, S // 2, 128), U32),
            pltpu.VMEM((NC, HA, DA // 2, KC), U32),
            [pltpu.VMEM((S, QT), F32)] * RING,
            pltpu.SMEM((2,), jnp.int32),
            pltpu.VMEM((LAG, 8, QT), F32),
            pltpu.VMEM((8 * DA, QT), F32),
            pltpu.VMEM((2, D // 128, QT // 2, 128), U32),
            pltpu.VMEM((L, D), F32),
            pltpu.VMEM((L, HB * DB), F32),
            pltpu.VMEM((2, NCG, QT, CW), F32),
            pltpu.VMEM((QT + S, 128), F32),
            pltpu.VMEM((NCG, S, CW), BF16),
            pltpu.SemaphoreType.DMA((21,)),
            pltpu.SemaphoreType.DMA((2,)),
            pltpu.SemaphoreType.DMA(()),
        ],
        compiler_params=pltpu.CompilerParams(vmem_limit_bytes=110 * 1024 * 1024),
        name="gated_mix",
    )(
        A_x.reshape(S, D), A_wqkv, A_wo, B_mem0.reshape(MEM, D),
        B_Wq.reshape(D * HB, DB), B_Wk.reshape(D * HB, DB), B_Wv.reshape(D * HB, DB),
        B_Wo.reshape(HB * DB, D), gate_w.reshape(1, D),
    )
    return out.reshape(1, S, D)
```

```python
import math

import jax
import jax.numpy as jnp
import jax.experimental.pallas as pl
import jax.experimental.pallas.tpu as pltpu

CFG = {"order": "pQKSPVsvf", "ls": 1, "lv": 3, "end": [3, "s", "v", 8, "v", 13, "v", 32, "m"], "unroll": 1}
BF16, F32, U32 = jnp.bfloat16, jnp.float32, jnp.uint32
LOG2E = math.log2(math.e)

S, D = 2048, 1024
HA, DA = 32, 32
HB, DB = 32, 128
MEM, SEG = 8, 32
L = MEM + SEG
NSTEP = S // SEG
QT = 128
KC = 512
NC = S // KC
LAG = 2
RING = 4
CW = 256
NCG = D // CW
MC = 256
XB = 512
WA0 = 3 * HB
WCH = D * HB // 2 // NCG


def _bf(x):
    return pltpu.bitcast(x, BF16)


def _words(x):
    return pltpu.bitcast(x.astype(BF16), U32)


def _dot(a, b):
    return jnp.dot(a, b, preferred_element_type=F32)


def _dot_nt(a, b):
    return jax.lax.dot_general(a, b, (((1,), (1,)), ((), ())), preferred_element_type=F32)


def _recip(x):
    r = pltpu.reciprocal(x, approx=True)
    return r * (2.0 - x * r)


def _rows(start, n):
    return pl.ds(pl.multiple_of(start, n), n)


def _transpose8(v):
    sub = jax.lax.broadcasted_iota(U32, (8, 128), 0)
    for s in (4, 2, 1):
        keep = (sub & s) == 0
        nv = list(v)
        for i in range(8):
            if i & s == 0:
                a, b = v[i], v[i + s]
                nv[i] = jnp.where(keep, a, pltpu.roll(b, s, 0))
                nv[i + s] = jnp.where(keep, pltpu.roll(a, 8 - s, 0), b)
        v = nv
    return v


def _kernel(x_hbm, wa_hbm, woa_hbm, mem_ref, wq_hbm, wk_hbm, wv_hbm, wob_hbm, gw_ref, out_hbm,
            xs, wt, woa, wob, stage, ka, qa, vt, sbuf, zero, mcar, ot, oa,
            hbuf, obuf, bbuf, gbuf, outb, x_sem, wa_sem, woa_sem, wob_sem, st_sem, out_sem):

    b_weights = (wq_hbm, wk_hbm, wv_hbm)

    def x_copy(r):
        rows = pl.ds(r * XB // 2, XB // 2)
        return pltpu.make_async_copy(x_hbm.bitcast(U32).at[rows], xs.at[rows], x_sem.at[r])

    def wa_copies(n):
        return [pltpu.make_async_copy(
            wa_hbm.bitcast(U32).at[:, _rows(t * 128, 128)], wt.at[WA0 + t], wa_sem.at[n])
            for t in (2 * n, 2 * n + 1)]

    def woa_copy(n):
        return pltpu.make_async_copy(
            woa_hbm.bitcast(U32).at[:, _rows(n * CW, CW)], woa.at[n], woa_sem.at[n])

    def wob_copy(n):
        rows = _rows(n * (HB * DB // 8), HB * DB // 8)
        return pltpu.make_async_copy(wob_hbm.bitcast(U32).at[rows], wob.at[rows], wob_sem.at[n])

    def stage_copy(part, n):
        rows = _rows(n * WCH, WCH)
        return pltpu.make_async_copy(
            b_weights[part].bitcast(U32).at[rows], stage.at[part, rows], st_sem.at[part * NCG + n])

    def out_copy(qtile, cg):
        rows = _rows(qtile * QT, QT)
        return pltpu.make_async_copy(
            outb.at[cg, rows], out_hbm.at[rows, _rows(cg * CW, CW)], out_sem)

    def weights(tile, n):
        return jnp.concatenate([_bf(wt[tile + t]) for t in range(n)], axis=1)

    for cp in wa_copies(0):
        cp.start()
    x_copy(0).start()
    x_copy(1).start()

    for i in range(RING - LAG, RING):
        sbuf[i][...] = jnp.zeros((S, QT), F32)
    mcar[...] = jnp.zeros(mcar.shape, F32)
    ot[...] = jnp.zeros(ot.shape, F32)
    oa[1] = jnp.zeros(oa.shape[1:], U32)
    bbuf[1] = jnp.zeros(bbuf.shape[1:], F32)
    gbuf[0:QT, :] = jnp.zeros((QT, 128), F32)
    zero[0] = 0
    gw = jnp.broadcast_to(gw_ref[...].astype(F32), (8, D))

    def load_segment(seg):
        xr = _bf(xs[_rows(seg * (SEG // 2), SEG // 2), :]).astype(F32)
        hbuf[MEM:L, :] = xr
        z = jnp.sum(xr.reshape(SEG // 8, 8, D) * gw, axis=-1, keepdims=True).reshape(SEG, 1)
        gbuf[_rows(QT + seg * SEG, SEG), :] = jnp.broadcast_to(
            1.0 / (1.0 + jnp.exp(-z)), (SEG, 128))

    def relayout(part, group):
        w = stage[part, _rows(group * 16 * HB // 2, 16 * HB // 2), :].reshape(8, 2, HB // 2, 128)
        a, b = w[:, 0], w[:, 1]
        lo = (a & U32(0xFFFF)) | (b << 16)
        hi = (a >> 16) | (b & U32(0xFFFF0000))
        rows = _rows(group * 8, 8)
        for par, t in enumerate((lo, hi)):
            for half in range(2):
                v = _transpose8([t[i, half * 8:(half + 1) * 8, :] for i in range(8)])
                for jj in range(8):
                    wt[3 * (2 * (half * 8 + jj) + par) + part, rows, :] = v[jj]

    def project(part, tile, m):
        y = _dot(_bf(xs[m * MC // 2:(m + 1) * MC // 2, :]),
                 weights(WA0 + part * (D // 128) + tile, 1))
        if part == 2:
            col = (m * MC) % KC
            vt[(m * MC) // KC, pl.ds(tile * (128 // DA), 128 // DA), :, col:col + MC] = (
                _words(y.T).reshape(128 // DA, DA // 2, MC))
        elif part == 1:
            ka[tile, m * MC // 2:(m + 1) * MC // 2, :] = _words(y)
        else:
            qa[tile, m * MC // 2:(m + 1) * MC // 2, :] = _words(y * (DA ** -0.5 * LOG2E))

    starts = ([x_copy(2)], [x_copy(3)], wa_copies(1) + [stage_copy(0, 0)],
              wa_copies(2) + [stage_copy(0, 1)])
    for r in range(S // XB):
        x_copy(r).wait()
        if r == 0:
            for cp in wa_copies(0):
                cp.wait()
            hbuf[0:MEM, :] = mem_ref[...].astype(F32)
            load_segment(0)
        for cp in starts[r]:
            cp.start()
        for m in range(r * XB // MC, (r + 1) * XB // MC):
            project(0, 0, m)
            project(0, 1, m)

    for part in range(3):
        def proj_body(n, carry, part=part):
            cur = part * NCG + n
            chunk = n - 1 if part == 0 else n
            for cp in wa_copies(cur):
                cp.wait()
            stage_copy(part, chunk).wait()

            @pl.when(cur + 2 < 3 * NCG)
            def _():
                for cp in wa_copies(cur + 2):
                    cp.start()

            ahead = chunk + 2 - (NCG - 1 if part == 0 else NCG)

            @pl.when(ahead < 0)
            def _():
                stage_copy(part, chunk + 2).start()

            if part < 2:
                @pl.when(ahead >= 0)
                def _():
                    stage_copy(part + 1, ahead).start()
            if part == 1:
                wob_copy(n).start()
            if part == 2:
                woa_copy(n).start()

            for g in range(16):
                project(part, 2 * n + g % 2, g // 2)
                relayout(part, chunk * 16 + g)
                if part == 2 and g % 4 == 1:
                    relayout(0, (NCG - 1) * 16 + 4 * n + g // 4)
            return carry

        if part == 1:
            stage_copy(0, NCG - 1).start()
        if part == 2:
            stage_copy(0, NCG - 1).wait()
        jax.lax.fori_loop(1 if part == 0 else 0, NCG, proj_body, 0)

    for n in range(NCG):
        woa_copy(n).wait()
        wob_copy(n).wait()

    row = jax.lax.broadcasted_iota(jnp.int32, (L, L), 0)
    col = jax.lax.broadcasted_iota(jnp.int32, (L, L), 1)
    mask_b = (row < MEM) | (row >= col)
    head_lane = jax.lax.broadcasted_iota(jnp.int32, (QT // 2, 128), 1) // DA

    def a_scores(tile, qtile, i, c):
        q = qa[tile, _rows(qtile * (QT // 2), QT // 2), :]
        q = _bf(jnp.where(head_lane == i % 4, q, U32(0)))
        mx = None
        n = KC // 4
        for r in range(c * KC, (c + 1) * KC, n):
            st = _dot_nt(_bf(ka[tile, r // 2:(r + n) // 2, :]), q)
            sbuf[i % RING][r:r + n, :] = st
            m = st.reshape(n // 8, 8, 128).max(axis=0)
            mx = m if mx is None else jnp.maximum(mx, m)
        return mx

    def a_probs(i, c, m):
        p = jnp.exp2(sbuf[i % RING][_rows(zero[0] + c * KC, KC), :] - m)
        return p.astype(BF16), p.reshape(KC // 8, 8, 128).sum(axis=0)

    def a_values(head, c, p):
        return _dot(_bf(vt[c, head]), p)

    def a_finish(i, acc, den):
        ot[i * DA:(i + 1) * DA, :] = acc * _recip(jnp.sum(den, axis=0, keepdims=True))

    def a_transpose(qtile, tile, which):
        oa[qtile % 2, tile] = _words(ot[which * 128:(which + 1) * 128, :].T)

    def mix(qtile, cg):
        o = jnp.concatenate([_bf(oa[qtile % 2, t]) for t in range(D // 128)], axis=1)
        a = _dot(o, _bf(woa[cg]))
        g = gbuf[_rows((qtile + 1) * QT, QT), :]
        g = jnp.concatenate([g] * (CW // 128), axis=1)
        outb[cg, _rows(jnp.maximum(qtile, 0) * QT, QT), :] = (
            g * a + (1.0 - g) * bbuf[qtile % 2, cg]).astype(BF16)

    def b_out(h0, h1):
        return _dot(obuf[:, h0 * DB:h1 * DB], _bf(wob[h0 * DB // 2:h1 * DB // 2, :]))

    def b_scores(q, k):
        sc = jnp.where(mask_b, _dot_nt(q, k), -1e9 * LOG2E)
        pr = jnp.exp2(sc - jnp.max(sc, axis=-1, keepdims=True))
        return pr * _recip(jnp.sum(pr, axis=-1, keepdims=True))

    def b_values(hd, pr, v):
        obuf[:, hd * DB:(hd + 1) * DB] = _dot(pr, v)

    def step(s):
        qtile, cg = s // 4, s % 4
        cg_prev = (s + 3) % 4
        maxes = {i - LAG: mcar[i, 0:1, :] for i in range(LAG)}
        qs, ks, vs, prs = {}, {}, {}, {}
        for h in range(HB):
            i, c = h // NC, h % NC
            ip = i - LAG
            for op in CFG["order"]:
                if op == "p":
                    p, den = a_probs(ip, c, maxes[ip])
                    dsum = den if c == 0 else dsum + den
                elif op == "X":
                    y = _dot(hbuf[...], weights(3 * h, 3))
                    qs[h] = y[:, :DB] * (DB ** -0.5 * LOG2E)
                    ks[h] = y[:, DB:2 * DB].astype(BF16)
                    vs[h] = y[:, 2 * DB:].astype(BF16)
                elif op == "Q":
                    qs[h] = _dot(hbuf[...], weights(3 * h, 1)) * (DB ** -0.5 * LOG2E)
                elif op == "K":
                    ks[h] = _dot(hbuf[...], weights(3 * h + 1, 1)).astype(BF16)
                elif op == "V":
                    vs[h] = _dot(hbuf[...], weights(3 * h + 2, 1)).astype(BF16)
                elif op == "S":
                    mx = a_scores(2 * cg + i // 4, qtile, i, c)
                    m_run = mx if c == 0 else jnp.maximum(m_run, mx)
                elif op == "P":
                    o = a_values(8 * cg + ip if ip >= 0 else 8 * cg_prev + 8 + ip, c, p)
                    acc = o if c == 0 else acc + o
                elif op == "s":
                    if h >= CFG["ls"]:
                        prs[h - CFG["ls"]] = b_scores(qs.pop(h - CFG["ls"]), ks.pop(h - CFG["ls"]))
                elif op == "v":
                    if h >= CFG["lv"]:
                        b_values(h - CFG["lv"], prs.pop(h - CFG["lv"]), vs.pop(h - CFG["lv"]))
                elif op == "f" and c == NC - 1:
                    a_finish(ip % 8, acc, dsum)
                    maxes[i] = jnp.max(m_run, axis=0, keepdims=True)
                    if ip == -1:
                        a_transpose((s + 7) // 4, 2 * cg_prev + 1, 1)
                    if ip == 3:
                        a_transpose(qtile, 2 * cg, 0)
        for i in range(LAG):
            mcar[i] = jnp.broadcast_to(maxes[8 - LAG + i], (8, QT))

        load_segment(jnp.minimum(s + 1, NSTEP - 1))
        y = None
        h0 = 0
        for op in CFG["end"]:
            if op == "s":
                hd = min(qs)
                prs[hd] = b_scores(qs.pop(hd), ks.pop(hd))
            elif op == "v":
                hd = min(prs)
                b_values(hd, prs.pop(hd), vs.pop(hd))
            elif op == "m":
                mix(qtile - 1, cg)
            else:
                t = b_out(h0, op)
                y = t if y is None else y + t
                h0 = op
        assert h0 == HB and not prs and not qs
        hbuf[0:MEM, :] = y[0:MEM].astype(BF16).astype(F32)
        for t in range(NCG):
            bbuf[qtile % 2, t, _rows(cg * SEG, SEG), :] = y[MEM:L, t * CW:(t + 1) * CW]

    U = CFG["unroll"]

    def steps(t, carry):
        for u in range(U):
            step(U * t + u)

        @pl.when(t >= 4 // U)
        def _():
            for u in range(U):
                out_copy((U * t) // 4 - 1, (U * t) % 4 + u).start()
        return carry

    jax.lax.fori_loop(0, NSTEP // U, steps, 0)

    for i in range(LAG):
        for c in range(NC):
            p, den = a_probs(i - LAG, c, mcar[i, 0:1, :])
            o = a_values(HA - LAG + i, c, p)
            acc, dsum = (o, den) if c == 0 else (acc + o, dsum + den)
        a_finish(8 - LAG + i, acc, dsum)
    last = S // QT - 1
    a_transpose(last, D // 128 - 1, 1)
    for cg in range(NCG):
        mix(last, cg)
        out_copy(last, cg).start()

    def drain(t, carry):
        out_copy(t // NCG, t % NCG).wait()
        return carry

    jax.lax.fori_loop(0, (S // QT) * NCG, drain, 0)


@jax.jit
def pallas_gated_mix__softmax_full_mha__memory_aug_recurrent_mem_tr__prompt_kernel(
    A_x: jax.Array,
    A_wqkv: jax.Array,
    A_wo: jax.Array,
    B_x: jax.Array,
    B_mem0: jax.Array,
    B_Wq: jax.Array,
    B_Wk: jax.Array,
    B_Wv: jax.Array,
    B_Wo: jax.Array,
    B_seg_len: jax.Array,
    gate_w: jax.Array,
):
    del B_x, B_seg_len
    assert A_x.shape == (1, S, D) and B_mem0.shape == (1, MEM, D) and B_Wq.shape == (D, HB, DB)

    hbm = pl.BlockSpec(memory_space=pl.ANY)
    vmem = pl.BlockSpec(memory_space=pltpu.VMEM)
    out = pl.pallas_call(
        _kernel,
        out_shape=jax.ShapeDtypeStruct((S, D), BF16),
        in_specs=[hbm, hbm, hbm, vmem, hbm, hbm, hbm, hbm, vmem],
        out_specs=hbm,
        scratch_shapes=[
            pltpu.VMEM((S // 2, D), U32),
            pltpu.VMEM((WA0 + 3 * D // 128, D // 2, 128), U32),
            pltpu.VMEM((NCG, D // 2, CW), U32),
            pltpu.VMEM((HB * DB // 2, D), U32),
            pltpu.VMEM((3, D * HB // 2, DB), U32),
            pltpu.VMEM((D // 128, S // 2, 128), U32),
            pltpu.VMEM((D // 128, S // 2, 128), U32),
            pltpu.VMEM((NC, HA, DA // 2, KC), U32),
            [pltpu.VMEM((S, QT), F32)] * RING,
            pltpu.SMEM((1,), jnp.int32),
            pltpu.VMEM((LAG, 8, QT), F32),
            pltpu.VMEM((8 * DA, QT), F32),
            pltpu.VMEM((2, D // 128, QT // 2, 128), U32),
            pltpu.VMEM((L, D), F32),
            pltpu.VMEM((L, HB * DB), F32),
            pltpu.VMEM((2, NCG, QT, CW), F32),
            pltpu.VMEM((QT + S, 128), F32),
            pltpu.VMEM((NCG, S, CW), BF16),
            pltpu.SemaphoreType.DMA((S // XB,)),
            pltpu.SemaphoreType.DMA((3 * NCG,)),
            pltpu.SemaphoreType.DMA((NCG,)),
            pltpu.SemaphoreType.DMA((NCG,)),
            pltpu.SemaphoreType.DMA((3 * NCG,)),
            pltpu.SemaphoreType.DMA(()),
        ],
        compiler_params=pltpu.CompilerParams(vmem_limit_bytes=110 * 1024 * 1024),
        name="gated_mix",
    )(
        A_x.reshape(S, D), A_wqkv, A_wo, B_mem0.reshape(MEM, D),
        B_Wq.reshape(D * HB, DB), B_Wk.reshape(D * HB, DB), B_Wv.reshape(D * HB, DB),
        B_Wo.reshape(HB * DB, D), gate_w.reshape(1, D),
    )
    return out.reshape(1, S, D)
```

```python
import math

import jax
import jax.numpy as jnp
import jax.experimental.pallas as pl
import jax.experimental.pallas.tpu as pltpu

CFG = {'order': 'QpKSVPsvf', 'ls': 1, 'lv': 3, 'end': [3, 's', 'v', 8, 'v', 13, 'v', 32, 'm'], 'unroll': 2, 'sw': 16}
BF16, F32, U32 = jnp.bfloat16, jnp.float32, jnp.uint32
LOG2E = math.log2(math.e)

S, D = 2048, 1024
HA, DA = 32, 32
HB, DB = 32, 128
MEM, SEG = 8, 32
L = MEM + SEG
NSTEP = S // SEG
QT = 128
KC = 512
NC = S // KC
LAG = 2
RING = 4
CW = 256
NCG = D // CW
MC = 256
XB = 512
WA0 = 3 * HB
WCH = D * HB // 2 // NCG


def _bf(x):
    return pltpu.bitcast(x, BF16)


def _words(x):
    return pltpu.bitcast(x.astype(BF16), U32)


def _dot(a, b):
    return jnp.dot(a, b, preferred_element_type=F32)


def _dot_nt(a, b):
    return jax.lax.dot_general(a, b, (((1,), (1,)), ((), ())), preferred_element_type=F32)


def _recip(x):
    r = pltpu.reciprocal(x, approx=True)
    return r * (2.0 - x * r)


def _rows(start, n):
    return pl.ds(pl.multiple_of(start, n), n)


def _transpose8(v):
    sub = jax.lax.broadcasted_iota(U32, (8, 128), 0)
    for s in (4, 2, 1):
        keep = (sub & s) == 0
        nv = list(v)
        for i in range(8):
            if i & s == 0:
                a, b = v[i], v[i + s]
                nv[i] = jnp.where(keep, a, pltpu.roll(b, s, 0))
                nv[i + s] = jnp.where(keep, pltpu.roll(a, 8 - s, 0), b)
        v = nv
    return v


def _kernel(x_hbm, wa_hbm, woa_hbm, mem_ref, wq_hbm, wk_hbm, wv_hbm, wob_hbm, gw_ref, out_hbm,
            xs, wt, woa, wob, stage, ka, qa, vt, sbuf, zero, mcar, ot, oa,
            hbuf, obuf, bbuf, gbuf, outb, x_sem, wa_sem, woa_sem, wob_sem, st_sem, out_sem):

    b_weights = (wq_hbm, wk_hbm, wv_hbm)

    def x_copy(r):
        rows = pl.ds(r * XB // 2, XB // 2)
        return pltpu.make_async_copy(x_hbm.bitcast(U32).at[rows], xs.at[rows], x_sem.at[r])

    def wa_copies(n):
        return [pltpu.make_async_copy(
            wa_hbm.bitcast(U32).at[:, _rows(t * 128, 128)], wt.at[WA0 + t], wa_sem.at[n])
            for t in (2 * n, 2 * n + 1)]

    def woa_copy(n):
        return pltpu.make_async_copy(
            woa_hbm.bitcast(U32).at[:, _rows(n * CW, CW)], woa.at[n], woa_sem.at[n])

    def wob_copy(n):
        rows = _rows(n * (HB * DB // 8), HB * DB // 8)
        return pltpu.make_async_copy(wob_hbm.bitcast(U32).at[rows], wob.at[rows], wob_sem.at[n])

    def stage_copy(part, n):
        rows = _rows(n * WCH, WCH)
        return pltpu.make_async_copy(
            b_weights[part].bitcast(U32).at[rows], stage.at[part, rows], st_sem.at[part * NCG + n])

    def out_copy(qtile, cg):
        rows = _rows(qtile * QT, QT)
        return pltpu.make_async_copy(
            outb.at[cg, rows], out_hbm.at[rows, _rows(cg * CW, CW)], out_sem)

    def weights(tile, n):
        return jnp.concatenate([_bf(wt[tile + t]) for t in range(n)], axis=1)

    for cp in wa_copies(0):
        cp.start()
    x_copy(0).start()
    x_copy(1).start()

    for i in range(RING - LAG, RING):
        sbuf[i][...] = jnp.zeros((S, QT), F32)
    mcar[...] = jnp.zeros(mcar.shape, F32)
    ot[...] = jnp.zeros(ot.shape, F32)
    oa[1] = jnp.zeros(oa.shape[1:], U32)
    bbuf[1] = jnp.zeros(bbuf.shape[1:], F32)
    gbuf[0:QT, :] = jnp.zeros((QT, 128), F32)
    zero[0] = 0
    gw = jnp.broadcast_to(gw_ref[...].astype(F32), (8, D))

    def load_segment(seg):
        xr = _bf(xs[_rows(seg * (SEG // 2), SEG // 2), :]).astype(F32)
        hbuf[MEM:L, :] = xr
        z = jnp.sum(xr.reshape(SEG // 8, 8, D) * gw, axis=-1, keepdims=True).reshape(SEG, 1)
        gbuf[_rows(QT + seg * SEG, SEG), :] = jnp.broadcast_to(
            1.0 / (1.0 + jnp.exp(-z)), (SEG, 128))

    def relayout(part, group):
        w = stage[part, _rows(group * 16 * HB // 2, 16 * HB // 2), :].reshape(8, 2, HB // 2, 128)
        a, b = w[:, 0], w[:, 1]
        lo = (a & U32(0xFFFF)) | (b << 16)
        hi = (a >> 16) | (b & U32(0xFFFF0000))
        rows = _rows(group * 8, 8)
        for par, t in enumerate((lo, hi)):
            for half in range(2):
                v = _transpose8([t[i, half * 8:(half + 1) * 8, :] for i in range(8)])
                for jj in range(8):
                    wt[3 * (2 * (half * 8 + jj) + par) + part, rows, :] = v[jj]

    def project(part, tile, m):
        y = _dot(_bf(xs[m * MC // 2:(m + 1) * MC // 2, :]),
                 weights(WA0 + part * (D // 128) + tile, 1))
        if part == 2:
            col = (m * MC) % KC
            vt[(m * MC) // KC, pl.ds(tile * (128 // DA), 128 // DA), :, col:col + MC] = (
                _words(y.T).reshape(128 // DA, DA // 2, MC))
        elif part == 1:
            ka[tile, m * MC // 2:(m + 1) * MC // 2, :] = _words(y)
        else:
            qa[tile, m * MC // 2:(m + 1) * MC // 2, :] = _words(y * (DA ** -0.5 * LOG2E))

    starts = ([x_copy(2)], [x_copy(3)], wa_copies(1) + [stage_copy(0, 0)],
              wa_copies(2) + [stage_copy(0, 1)])
    for r in range(S // XB):
        x_copy(r).wait()
        if r == 0:
            for cp in wa_copies(0):
                cp.wait()
            hbuf[0:MEM, :] = mem_ref[...].astype(F32)
            load_segment(0)
        for cp in starts[r]:
            cp.start()
        for m in range(r * XB // MC, (r + 1) * XB // MC):
            project(0, 0, m)
            project(0, 1, m)

    for part in range(3):
        def proj_body(n, carry, part=part):
            cur = part * NCG + n
            chunk = n - 1 if part == 0 else n
            for cp in wa_copies(cur):
                cp.wait()
            stage_copy(part, chunk).wait()

            @pl.when(cur + 2 < 3 * NCG)
            def _():
                for cp in wa_copies(cur + 2):
                    cp.start()

            ahead = chunk + 2 - (NCG - 1 if part == 0 else NCG)

            @pl.when(ahead < 0)
            def _():
                stage_copy(part, chunk + 2).start()

            if part < 2:
                @pl.when(ahead >= 0)
                def _():
                    stage_copy(part + 1, ahead).start()
            if part == 1:
                wob_copy(n).start()
            if part == 2:
                woa_copy(n).start()

            for g in range(16):
                project(part, 2 * n + g % 2, g // 2)
                relayout(part, chunk * 16 + g)
                if part == 2 and g % 4 == 1:
                    relayout(0, (NCG - 1) * 16 + 4 * n + g // 4)
            return carry

        if part == 1:
            stage_copy(0, NCG - 1).start()
        if part == 2:
            stage_copy(0, NCG - 1).wait()
        jax.lax.fori_loop(1 if part == 0 else 0, NCG, proj_body, 0)

    for n in range(NCG):
        woa_copy(n).wait()
        wob_copy(n).wait()

    row = jax.lax.broadcasted_iota(jnp.int32, (L, L), 0)
    col = jax.lax.broadcasted_iota(jnp.int32, (L, L), 1)
    mask_b = (row < MEM) | (row >= col)
    head_lane = jax.lax.broadcasted_iota(jnp.int32, (QT // 2, 128), 1) // DA

    def a_scores(tile, qtile, i, c):
        q = qa[tile, _rows(qtile * (QT // 2), QT // 2), :]
        q = _bf(jnp.where(head_lane == i % 4, q, U32(0)))
        mx = None
        n = KC // 4
        for r in range(c * KC, (c + 1) * KC, n):
            st = _dot_nt(_bf(ka[tile, r // 2:(r + n) // 2, :]), q)
            sbuf[i % RING][r:r + n, :] = st
            m = st.reshape(n // 8, 8, 128).max(axis=0)
            mx = m if mx is None else jnp.maximum(mx, m)
        return mx

    def not_before(x, other):
        nop = pltpu.bitcast(other[0:8, 0:QT], U32) & zero[0].astype(U32)
        return pltpu.bitcast(pltpu.bitcast(x, U32) | nop, F32)

    def a_probs(i, c, m):
        st = sbuf[i % RING][_rows(zero[0] + c * KC, KC), :].reshape(KC // 8, 8, QT)
        p = jnp.exp2(st - m).reshape(KC, QT)
        W = CFG["sw"]
        return p.astype(BF16), p.reshape(KC // W, W, 128).sum(axis=0)

    def a_values(head, c, p):
        return _dot(_bf(vt[c, head]), p)

    def a_finish(i, acc, den):
        ot[i * DA:(i + 1) * DA, :] = acc * _recip(jnp.sum(den, axis=0, keepdims=True))

    def a_transpose(qtile, tile, which):
        oa[qtile % 2, tile] = _words(ot[which * 128:(which + 1) * 128, :].T)

    def mix(qtile, cg):
        o = jnp.concatenate([_bf(oa[qtile % 2, t]) for t in range(D // 128)], axis=1)
        a = _dot(o, _bf(woa[cg]))
        g = gbuf[_rows((qtile + 1) * QT, QT), :]
        g = jnp.concatenate([g] * (CW // 128), axis=1)
        outb[cg, _rows(jnp.maximum(qtile, 0) * QT, QT), :] = (
            g * a + (1.0 - g) * bbuf[qtile % 2, cg]).astype(BF16)

    def b_out(h0, h1):
        return _dot(obuf[:, h0 * DB:h1 * DB], _bf(wob[h0 * DB // 2:h1 * DB // 2, :]))

    def b_scores(q, k):
        sc = jnp.where(mask_b, _dot_nt(q, k), -1e9 * LOG2E)
        pr = jnp.exp2(sc - jnp.max(sc, axis=-1, keepdims=True))
        return pr * _recip(jnp.sum(pr, axis=-1, keepdims=True))

    def b_values(hd, pr, v):
        obuf[:, hd * DB:(hd + 1) * DB] = _dot(pr, v)

    def step(s):
        qtile, cg = s // 4, s % 4
        cg_prev = (s + 3) % 4
        maxes = {i - LAG: mcar[i] for i in range(LAG)}
        qs, ks, vs, prs = {}, {}, {}, {}
        last = None
        for h in range(HB):
            i, c = h // NC, h % NC
            ip = i - LAG
            for op in CFG["order"]:
                if op == "p":
                    m = maxes[ip]
                    if last is not None:
                        m = not_before(m, last)
                    p, den = a_probs(ip, c, m)
                    dsum = den if c == 0 else dsum + den
                elif op == "X":
                    y = _dot(hbuf[...], weights(3 * h, 3))
                    qs[h] = y[:, :DB] * (DB ** -0.5 * LOG2E)
                    ks[h] = y[:, DB:2 * DB].astype(BF16)
                    vs[h] = y[:, 2 * DB:].astype(BF16)
                elif op == "Q":
                    last = _dot(hbuf[...], weights(3 * h, 1))
                    qs[h] = last * (DB ** -0.5 * LOG2E)
                elif op == "K":
                    last = _dot(hbuf[...], weights(3 * h + 1, 1))
                    ks[h] = last.astype(BF16)
                elif op == "V":
                    last = _dot(hbuf[...], weights(3 * h + 2, 1))
                    vs[h] = last.astype(BF16)
                elif op == "S":
                    mx = a_scores(2 * cg + i // 4, qtile, i, c)
                    m_run = mx if c == 0 else jnp.maximum(m_run, mx)
                elif op == "P":
                    o = a_values(8 * cg + ip if ip >= 0 else 8 * cg_prev + 8 + ip, c, p)
                    acc = o if c == 0 else acc + o
                elif op == "s":
                    if h >= CFG["ls"]:
                        prs[h - CFG["ls"]] = b_scores(qs.pop(h - CFG["ls"]), ks.pop(h - CFG["ls"]))
                elif op == "v":
                    if h >= CFG["lv"]:
                        b_values(h - CFG["lv"], prs.pop(h - CFG["lv"]), vs.pop(h - CFG["lv"]))
                elif op == "f" and c == NC - 1:
                    a_finish(ip % 8, acc, dsum)
                    maxes[i] = jnp.broadcast_to(jnp.max(m_run, axis=0, keepdims=True), (8, QT))
                    if ip == -1:
                        a_transpose((s + 7) // 4, 2 * cg_prev + 1, 1)
                    if ip == 3:
                        a_transpose(qtile, 2 * cg, 0)
        for i in range(LAG):
            mcar[i] = maxes[8 - LAG + i]

        load_segment(jnp.minimum(s + 1, NSTEP - 1))
        y = None
        h0 = 0
        for op in CFG["end"]:
            if op == "s":
                hd = min(qs)
                prs[hd] = b_scores(qs.pop(hd), ks.pop(hd))
            elif op == "v":
                hd = min(prs)
                b_values(hd, prs.pop(hd), vs.pop(hd))
            elif op == "m":
                mix(qtile - 1, cg)
            else:
                t = b_out(h0, op)
                y = t if y is None else y + t
                h0 = op
        assert h0 == HB and not prs and not qs
        hbuf[0:MEM, :] = y[0:MEM].astype(BF16).astype(F32)
        for t in range(NCG):
            bbuf[qtile % 2, t, _rows(cg * SEG, SEG), :] = y[MEM:L, t * CW:(t + 1) * CW]

    U = CFG["unroll"]

    def steps(t, carry):
        for u in range(U):
            step(U * t + u)

        @pl.when(t >= 4 // U)
        def _():
            for u in range(U):
                out_copy((U * t) // 4 - 1, (U * t) % 4 + u).start()
        return carry

    jax.lax.fori_loop(0, NSTEP // U, steps, 0)

    for i in range(LAG):
        for c in range(NC):
            p, den = a_probs(i - LAG, c, mcar[i])
            o = a_values(HA - LAG + i, c, p)
            acc, dsum = (o, den) if c == 0 else (acc + o, dsum + den)
        a_finish(8 - LAG + i, acc, dsum)
    last = S // QT - 1
    a_transpose(last, D // 128 - 1, 1)
    for cg in range(NCG):
        mix(last, cg)
        out_copy(last, cg).start()

    def drain(t, carry):
        out_copy(t // NCG, t % NCG).wait()
        return carry

    jax.lax.fori_loop(0, (S // QT) * NCG, drain, 0)


@jax.jit
def pallas_gated_mix__softmax_full_mha__memory_aug_recurrent_mem_tr__prompt_kernel(
    A_x: jax.Array,
    A_wqkv: jax.Array,
    A_wo: jax.Array,
    B_x: jax.Array,
    B_mem0: jax.Array,
    B_Wq: jax.Array,
    B_Wk: jax.Array,
    B_Wv: jax.Array,
    B_Wo: jax.Array,
    B_seg_len: jax.Array,
    gate_w: jax.Array,
):
    del B_x, B_seg_len
    assert A_x.shape == (1, S, D) and B_mem0.shape == (1, MEM, D) and B_Wq.shape == (D, HB, DB)

    hbm = pl.BlockSpec(memory_space=pl.ANY)
    vmem = pl.BlockSpec(memory_space=pltpu.VMEM)
    out = pl.pallas_call(
        _kernel,
        out_shape=jax.ShapeDtypeStruct((S, D), BF16),
        in_specs=[hbm, hbm, hbm, vmem, hbm, hbm, hbm, hbm, vmem],
        out_specs=hbm,
        scratch_shapes=[
            pltpu.VMEM((S // 2, D), U32),
            pltpu.VMEM((WA0 + 3 * D // 128, D // 2, 128), U32),
            pltpu.VMEM((NCG, D // 2, CW), U32),
            pltpu.VMEM((HB * DB // 2, D), U32),
            pltpu.VMEM((3, D * HB // 2, DB), U32),
            pltpu.VMEM((D // 128, S // 2, 128), U32),
            pltpu.VMEM((D // 128, S // 2, 128), U32),
            pltpu.VMEM((NC, HA, DA // 2, KC), U32),
            [pltpu.VMEM((S, QT), F32)] * RING,
            pltpu.SMEM((1,), jnp.int32),
            pltpu.VMEM((LAG, 8, QT), F32),
            pltpu.VMEM((8 * DA, QT), F32),
            pltpu.VMEM((2, D // 128, QT // 2, 128), U32),
            pltpu.VMEM((L, D), F32),
            pltpu.VMEM((L, HB * DB), F32),
            pltpu.VMEM((2, NCG, QT, CW), F32),
            pltpu.VMEM((QT + S, 128), F32),
            pltpu.VMEM((NCG, S, CW), BF16),
            pltpu.SemaphoreType.DMA((S // XB,)),
            pltpu.SemaphoreType.DMA((3 * NCG,)),
            pltpu.SemaphoreType.DMA((NCG,)),
            pltpu.SemaphoreType.DMA((NCG,)),
            pltpu.SemaphoreType.DMA((3 * NCG,)),
            pltpu.SemaphoreType.DMA(()),
        ],
        compiler_params=pltpu.CompilerParams(vmem_limit_bytes=110 * 1024 * 1024),
        name="gated_mix",
    )(
        A_x.reshape(S, D), A_wqkv, A_wo, B_mem0.reshape(MEM, D),
        B_Wq.reshape(D * HB, DB), B_Wk.reshape(D * HB, DB), B_Wv.reshape(D * HB, DB),
        B_Wo.reshape(HB * DB, D), gate_w.reshape(1, D),
    )
    return out.reshape(1, S, D)
```

```python
import math

import jax
import jax.numpy as jnp
import jax.experimental.pallas as pl
import jax.experimental.pallas.tpu as pltpu

CFG = {"order": "QpKSVPsvf", "ls": 1, "lv": 3, "end": [2, "s", "v", 9, "v", 16, "v", 32, "m"], "end2": [3, "s", "v", 8, "v", 13, "v", 28, "m", 32], "unroll": 2, "sw": 16}
BF16, F32, U32 = jnp.bfloat16, jnp.float32, jnp.uint32
LOG2E = math.log2(math.e)

S, D = 2048, 1024
HA, DA = 32, 32
HB, DB = 32, 128
MEM, SEG = 8, 32
L = MEM + SEG
NSTEP = S // SEG
QT = 128
KC = 512
NC = S // KC
LAG = 2
RING = 4
CW = 256
NCG = D // CW
MC = 256
XB = 512
WA0 = 3 * HB
WCH = D * HB // 2 // NCG


def _bf(x):
    return pltpu.bitcast(x, BF16)


def _words(x):
    return pltpu.bitcast(x.astype(BF16), U32)


def _dot(a, b):
    return jnp.dot(a, b, preferred_element_type=F32)


def _dot_nt(a, b):
    return jax.lax.dot_general(a, b, (((1,), (1,)), ((), ())), preferred_element_type=F32)


def _recip(x):
    r = pltpu.reciprocal(x, approx=True)
    return r * (2.0 - x * r)


def _rows(start, n):
    return pl.ds(pl.multiple_of(start, n), n)


def _transpose8(v):
    sub = jax.lax.broadcasted_iota(U32, (8, 128), 0)
    for s in (4, 2, 1):
        keep = (sub & s) == 0
        nv = list(v)
        for i in range(8):
            if i & s == 0:
                a, b = v[i], v[i + s]
                nv[i] = jnp.where(keep, a, pltpu.roll(b, s, 0))
                nv[i + s] = jnp.where(keep, pltpu.roll(a, 8 - s, 0), b)
        v = nv
    return v


def _kernel(x_hbm, wa_hbm, woa_hbm, mem_ref, wq_hbm, wk_hbm, wv_hbm, wob_hbm, gw_ref, out_hbm,
            xs, wt, woa, wob, stage, ka, qa, vt, sbuf, zero, mcar, ot, oa,
            hbuf, obuf, bbuf, gbuf, outb, x_sem, wa_sem, woa_sem, wob_sem, st_sem, out_sem):

    b_weights = (wq_hbm, wk_hbm, wv_hbm)

    def x_copy(r):
        rows = pl.ds(r * XB // 2, XB // 2)
        return pltpu.make_async_copy(x_hbm.bitcast(U32).at[rows], xs.at[rows], x_sem.at[r])

    def wa_copies(n):
        return [pltpu.make_async_copy(
            wa_hbm.bitcast(U32).at[:, _rows(t * 128, 128)], wt.at[WA0 + t], wa_sem.at[n])
            for t in (2 * n, 2 * n + 1)]

    def woa_copy(n):
        return pltpu.make_async_copy(
            woa_hbm.bitcast(U32).at[:, _rows(n * CW, CW)], woa.at[n], woa_sem.at[n])

    def wob_copy(n):
        rows = _rows(n * (HB * DB // 8), HB * DB // 8)
        return pltpu.make_async_copy(wob_hbm.bitcast(U32).at[rows], wob.at[rows], wob_sem.at[n])

    def stage_copy(part, n):
        rows = _rows(n * WCH, WCH)
        return pltpu.make_async_copy(
            b_weights[part].bitcast(U32).at[rows], stage.at[part, rows], st_sem.at[part * NCG + n])

    def out_copy(qtile, cg):
        rows = _rows(qtile * QT, QT)
        return pltpu.make_async_copy(
            outb.at[cg, rows], out_hbm.at[rows, _rows(cg * CW, CW)], out_sem)

    def weights(tile, n):
        return jnp.concatenate([_bf(wt[tile + t]) for t in range(n)], axis=1)

    for cp in wa_copies(0):
        cp.start()
    x_copy(0).start()
    x_copy(1).start()

    for i in range(RING - LAG, RING):
        sbuf[i][...] = jnp.zeros((S, QT), F32)
    mcar[...] = jnp.zeros(mcar.shape, F32)
    ot[...] = jnp.zeros(ot.shape, F32)
    oa[1] = jnp.zeros(oa.shape[1:], U32)
    bbuf[1] = jnp.zeros(bbuf.shape[1:], F32)
    gbuf[0:QT, :] = jnp.zeros((QT, 128), F32)
    zero[0] = 0
    gw = jnp.broadcast_to(gw_ref[...].astype(F32).reshape(1, D), (8, D))

    def load_segment(seg):
        xr = _bf(xs[_rows(seg * (SEG // 2), SEG // 2), :]).astype(F32)
        hbuf[MEM:L, :] = xr
        z = jnp.sum(xr.reshape(SEG // 8, 8, D) * gw, axis=-1, keepdims=True).reshape(SEG, 1)
        gbuf[_rows(QT + seg * SEG, SEG), :] = jnp.broadcast_to(
            1.0 / (1.0 + jnp.exp(-z)), (SEG, 128))

    def relayout(part, group, halves=(0, 1)):
        w = stage[part, _rows(group * 16 * HB // 2, 16 * HB // 2), :].reshape(8, 2, HB // 2, 128)
        rows = _rows(group * 8, 8)
        for half in halves:
            a, b = w[:, 0, half * 8:(half + 1) * 8], w[:, 1, half * 8:(half + 1) * 8]
            lo = (a & U32(0xFFFF)) | (b << 16)
            hi = (a >> 16) | (b & U32(0xFFFF0000))
            for odd, t in enumerate((lo, hi)):
                v = _transpose8([t[i] for i in range(8)])
                for j in range(8):
                    wt[3 * (2 * (half * 8 + j) + odd) + part, rows, :] = v[j]

    def project(part, tile, m):
        rows = _rows(m * (MC // 2), MC // 2)
        y = _dot(_bf(xs[rows, :]), weights(WA0 + part * (D // 128) + tile, 1))
        if part == 2:
            col = (m * MC) % KC
            vt[(m * MC) // KC, pl.ds(tile * (128 // DA), 128 // DA), :, col:col + MC] = (
                _words(y.T).reshape(128 // DA, DA // 2, MC))
        elif part == 1:
            ka[tile, rows, :] = _words(y)
        else:
            qa[tile, rows, :] = _words(y * (DA ** -0.5 * LOG2E))

    NX = S // XB
    waits = [[x_copy(r)] for r in range(NX)] + [wa_copies(1)]
    waits[0] += wa_copies(0)
    starts = [[x_copy(2)], [x_copy(3)], wa_copies(1), [stage_copy(0, 0)],
              wa_copies(2) + [stage_copy(0, 1)] + wa_copies(3)]

    def first_body(i, carry):
        for k, (ws, ss) in enumerate(zip(waits, starts)):
            @pl.when(i == k)
            def _(ws=ws, ss=ss):
                for cp in ws:
                    cp.wait()
                for cp in ss:
                    cp.start()

        for m in range(XB // MC):
            for t in range(2):
                project(0, 2 * (i // NX) + t, (i % NX) * (XB // MC) + m)
        return carry

    jax.lax.fori_loop(0, 2 * NX, first_body, 0)
    hbuf[0:MEM, :] = mem_ref[...].astype(F32)
    load_segment(0)

    for part in range(3):
        def proj_body(n, carry, part=part):
            cur = part * NCG + n
            chunk = n - 2 if part == 0 else n
            for cp in wa_copies(cur):
                cp.wait()
            stage_copy(part, chunk).wait()

            @pl.when(cur + 2 < 3 * NCG)
            def _():
                for cp in wa_copies(cur + 2):
                    cp.start()

            if part == 0:
                stage_copy(1, chunk).start()
            else:
                @pl.when(n + 2 < NCG)
                def _():
                    stage_copy(part, n + 2).start()

            if part == 1:
                @pl.when(n + 2 >= NCG)
                def _():
                    stage_copy(2, n + 2 - NCG).start()

                wob_copy(n).start()
            if part == 2:
                woa_copy(n).start()

            for g in range(16):
                project(part, 2 * n + g % 2, g // 2)
                relayout(part, chunk * 16 + g)
                if part > 0 and g % 2 == 0:
                    relayout(0, (1 + part) * 16 + 4 * n + g // 4, halves=(g // 2 % 2,))
            return carry

        if part < 2:
            stage_copy(0, 2 + part).start()
        if part > 0:
            stage_copy(0, 1 + part).wait()
        jax.lax.fori_loop(2 if part == 0 else 0, NCG, proj_body, 0)

    for n in range(NCG):
        woa_copy(n).wait()
        wob_copy(n).wait()

    row = jax.lax.broadcasted_iota(jnp.int32, (L, L), 0)
    col = jax.lax.broadcasted_iota(jnp.int32, (L, L), 1)
    mask_b = (row < MEM) | (row >= col)
    head_lane = jax.lax.broadcasted_iota(jnp.int32, (QT // 2, 128), 1) // DA

    def a_scores(tile, qtile, i, c):
        q = qa[tile, _rows(qtile * (QT // 2), QT // 2), :]
        q = _bf(jnp.where(head_lane == i % 4, q, U32(0)))
        mx = None
        n = KC // 4
        for r in range(c * KC, (c + 1) * KC, n):
            st = _dot_nt(_bf(ka[tile, r // 2:(r + n) // 2, :]), q)
            sbuf[i % RING][r:r + n, :] = st
            m = st.reshape(n // 8, 8, 128).max(axis=0)
            mx = m if mx is None else jnp.maximum(mx, m)
        return mx

    def not_before(x, other):
        nop = pltpu.bitcast(other[0:8, 0:QT], U32) & zero[0].astype(U32)
        return pltpu.bitcast(pltpu.bitcast(x, U32) | nop, F32)

    def a_probs(i, c, m):
        st = sbuf[i % RING][_rows(zero[0] + c * KC, KC), :].reshape(KC // 8, 8, QT)
        p = jnp.exp2(st - m).reshape(KC, QT)
        W = CFG["sw"]
        return p.astype(BF16), p.reshape(KC // W, W, 128).sum(axis=0)

    def a_values(head, c, p):
        return _dot(_bf(vt[c, head]), p)

    def a_finish(i, acc, den):
        ot[i * DA:(i + 1) * DA, :] = acc * _recip(jnp.sum(den, axis=0, keepdims=True))

    def a_transpose(qtile, tile, which):
        oa[qtile % 2, tile] = _words(ot[which * 128:(which + 1) * 128, :].T)

    def mix(qtile, cg):
        o = jnp.concatenate([_bf(oa[qtile % 2, t]) for t in range(D // 128)], axis=1)
        a = _dot(o, _bf(woa[cg]))
        g = gbuf[_rows((qtile + 1) * QT, QT), :]
        g = jnp.concatenate([g] * (CW // 128), axis=1)
        outb[cg, _rows(jnp.maximum(qtile, 0) * QT, QT), :] = (
            g * a + (1.0 - g) * bbuf[qtile % 2, cg]).astype(BF16)

    def b_out(h0, h1):
        return _dot(obuf[:, h0 * DB:h1 * DB], _bf(wob[h0 * DB // 2:h1 * DB // 2, :]))

    def b_scores(q, k):
        sc = jnp.where(mask_b, _dot_nt(q, k), -1e9 * LOG2E)
        pr = jnp.exp2(sc - jnp.max(sc, axis=-1, keepdims=True))
        return pr * _recip(jnp.sum(pr, axis=-1, keepdims=True))

    def b_values(hd, pr, v):
        obuf[:, hd * DB:(hd + 1) * DB] = _dot(pr, v)

    def step(s, final):
        qtile, cg = s // 4, s % 4
        cg_prev = (s + 3) % 4
        maxes = {i - LAG: mcar[i] for i in range(LAG)}
        qs, ks, vs, prs = {}, {}, {}, {}
        last = None
        for h in range(HB):
            i, c = h // NC, h % NC
            ip = i - LAG
            for op in CFG["order"]:
                if op == "p":
                    m = maxes[ip]
                    if last is not None:
                        m = not_before(m, last)
                    p, den = a_probs(ip, c, m)
                    dsum = den if c == 0 else dsum + den
                elif op == "X":
                    y = _dot(hbuf[...], weights(3 * h, 3))
                    qs[h] = y[:, :DB] * (DB ** -0.5 * LOG2E)
                    ks[h] = y[:, DB:2 * DB].astype(BF16)
                    vs[h] = y[:, 2 * DB:].astype(BF16)
                elif op == "Q":
                    last = _dot(hbuf[...], weights(3 * h, 1))
                    qs[h] = last * (DB ** -0.5 * LOG2E)
                elif op == "K":
                    last = _dot(hbuf[...], weights(3 * h + 1, 1))
                    ks[h] = last.astype(BF16)
                elif op == "V":
                    last = _dot(hbuf[...], weights(3 * h + 2, 1))
                    vs[h] = last.astype(BF16)
                elif op == "S":
                    mx = a_scores(2 * cg + i // 4, qtile, i, c)
                    m_run = mx if c == 0 else jnp.maximum(m_run, mx)
                elif op == "P":
                    o = a_values(8 * cg + ip if ip >= 0 else 8 * cg_prev + 8 + ip, c, p)
                    acc = o if c == 0 else acc + o
                elif op == "s":
                    if h >= CFG["ls"]:
                        prs[h - CFG["ls"]] = b_scores(qs.pop(h - CFG["ls"]), ks.pop(h - CFG["ls"]))
                elif op == "v":
                    if h >= CFG["lv"]:
                        b_values(h - CFG["lv"], prs.pop(h - CFG["lv"]), vs.pop(h - CFG["lv"]))
                elif op == "f" and c == NC - 1:
                    a_finish(ip % 8, acc, dsum)
                    maxes[i] = jnp.broadcast_to(jnp.max(m_run, axis=0, keepdims=True), (8, QT))
                    if ip == -1:
                        a_transpose((s + 7) // 4, 2 * cg_prev + 1, 1)
                    if ip == 3:
                        a_transpose(qtile, 2 * cg, 0)
        for i in range(LAG):
            mcar[i] = maxes[8 - LAG + i]

        load_segment(jnp.minimum(s + 1, NSTEP - 1))
        y = None
        h0 = 0
        for op in CFG["end2" if final else "end"]:
            if op == "s":
                hd = min(qs)
                prs[hd] = b_scores(qs.pop(hd), ks.pop(hd))
            elif op == "v":
                hd = min(prs)
                b_values(hd, prs.pop(hd), vs.pop(hd))
            elif op == "m":
                mix(qtile - 1, cg)
            else:
                t = b_out(h0, op)
                y = t if y is None else y + t
                h0 = op
        assert h0 == HB and not prs and not qs
        hbuf[0:MEM, :] = y[0:MEM].astype(BF16).astype(F32)
        for t in range(NCG):
            bbuf[qtile % 2, t, _rows(cg * SEG, SEG), :] = y[MEM:L, t * CW:(t + 1) * CW]

    U = CFG["unroll"]

    def steps(t, carry):
        for u in range(U):
            step(U * t + u, u == U - 1)

        @pl.when(t >= 4 // U)
        def _():
            for u in range(U):
                out_copy((U * t) // 4 - 1, (U * t) % 4 + u).start()
        return carry

    jax.lax.fori_loop(0, NSTEP // U, steps, 0)

    for i in range(LAG):
        for c in range(NC):
            p, den = a_probs(i - LAG, c, mcar[i])
            o = a_values(HA - LAG + i, c, p)
            acc, dsum = (o, den) if c == 0 else (acc + o, dsum + den)
        a_finish(8 - LAG + i, acc, dsum)
    last = S // QT - 1
    a_transpose(last, D // 128 - 1, 1)
    for cg in range(NCG):
        mix(last, cg)
        out_copy(last, cg).start()

    def drain(t, carry):
        out_copy(t // NCG, t % NCG).wait()
        return carry

    jax.lax.fori_loop(0, (S // QT) * NCG, drain, 0)


@jax.jit
def pallas_gated_mix__softmax_full_mha__memory_aug_recurrent_mem_tr__prompt_kernel(
    A_x: jax.Array,
    A_wqkv: jax.Array,
    A_wo: jax.Array,
    B_x: jax.Array,
    B_mem0: jax.Array,
    B_Wq: jax.Array,
    B_Wk: jax.Array,
    B_Wv: jax.Array,
    B_Wo: jax.Array,
    B_seg_len: jax.Array,
    gate_w: jax.Array,
):
    del B_x, B_seg_len
    assert A_x.shape == (1, S, D) and B_mem0.shape == (1, MEM, D) and B_Wq.shape == (D, HB, DB)

    hbm = pl.BlockSpec(memory_space=pl.ANY)
    vmem = pl.BlockSpec(memory_space=pltpu.VMEM)
    out = pl.pallas_call(
        _kernel,
        out_shape=jax.ShapeDtypeStruct((S, D), BF16),
        in_specs=[hbm, hbm, hbm, vmem, hbm, hbm, hbm, hbm, vmem],
        out_specs=hbm,
        scratch_shapes=[
            pltpu.VMEM((S // 2, D), U32),
            pltpu.VMEM((WA0 + 3 * D // 128, D // 2, 128), U32),
            pltpu.VMEM((NCG, D // 2, CW), U32),
            pltpu.VMEM((HB * DB // 2, D), U32),
            pltpu.VMEM((3, D * HB // 2, DB), U32),
            pltpu.VMEM((D // 128, S // 2, 128), U32),
            pltpu.VMEM((D // 128, S // 2, 128), U32),
            pltpu.VMEM((NC, HA, DA // 2, KC), U32),
            [pltpu.VMEM((S, QT), F32)] * RING,
            pltpu.SMEM((1,), jnp.int32),
            pltpu.VMEM((LAG, 8, QT), F32),
            pltpu.VMEM((8 * DA, QT), F32),
            pltpu.VMEM((2, D // 128, QT // 2, 128), U32),
            pltpu.VMEM((L, D), F32),
            pltpu.VMEM((L, HB * DB), F32),
            pltpu.VMEM((2, NCG, QT, CW), F32),
            pltpu.VMEM((QT + S, 128), F32),
            pltpu.VMEM((NCG, S, CW), BF16),
            pltpu.SemaphoreType.DMA((S // XB,)),
            pltpu.SemaphoreType.DMA((3 * NCG,)),
            pltpu.SemaphoreType.DMA((NCG,)),
            pltpu.SemaphoreType.DMA((NCG,)),
            pltpu.SemaphoreType.DMA((3 * NCG,)),
            pltpu.SemaphoreType.DMA(()),
        ],
        compiler_params=pltpu.CompilerParams(vmem_limit_bytes=110 * 1024 * 1024),
        name="gated_mix",
    )(
        A_x.reshape(S, D), A_wqkv, A_wo, B_mem0.reshape(MEM, D),
        B_Wq.reshape(D * HB, DB), B_Wk.reshape(D * HB, DB), B_Wv.reshape(D * HB, DB),
        B_Wo.reshape(HB * DB, D), gate_w,
    )
    return out.reshape(1, S, D)
```

```python
import math

import jax
import jax.numpy as jnp
import jax.experimental.pallas as pl
import jax.experimental.pallas.tpu as pltpu

BF16, F32, U32 = jnp.bfloat16, jnp.float32, jnp.uint32
LOG2E = math.log2(math.e)

S, D = 2048, 1024
HA, DA = 32, 32
HB, DB = 32, 128
MEM, SEG = 8, 32
L = MEM + SEG
NSTEP = S // SEG
QT = 128
KC = 512
NC = S // KC
NI = HB // NC
LAG = 2
RING = 4
CW = 256
NCG = D // CW
MC = 256
XB = 512
NX = S // XB
WA0 = 3 * HB
WCH = D * HB // 2 // NCG


def _bf(x):
    return pltpu.bitcast(x, BF16)


def _words(x):
    return pltpu.bitcast(x.astype(BF16), U32)


def _dot(a, b):
    return jnp.dot(a, b, preferred_element_type=F32)


def _dot_nt(a, b):
    return jax.lax.dot_general(a, b, (((1,), (1,)), ((), ())), preferred_element_type=F32)


def _recip(x):
    r = pltpu.reciprocal(x, approx=True)
    return r * (2.0 - x * r)


def _rows(start, n):
    return pl.ds(pl.multiple_of(start, n), n)


def _transpose8(v):
    sub = jax.lax.broadcasted_iota(U32, (8, 128), 0)
    for s in (4, 2, 1):
        keep = (sub & s) == 0
        nv = list(v)
        for i in range(8):
            if i & s == 0:
                a, b = v[i], v[i + s]
                nv[i] = jnp.where(keep, a, pltpu.roll(b, s, 0))
                nv[i + s] = jnp.where(keep, pltpu.roll(a, 8 - s, 0), b)
        v = nv
    return v


def _kernel(x_hbm, wa_hbm, woa_hbm, mem_ref, wq_hbm, wk_hbm, wv_hbm, wob_hbm, gw_ref, out_hbm,
            xs, wt, woa, wob, stage, ka, qa, vt, sbuf, zero, mcar, ot, oa,
            hbuf, obuf, bbuf, gbuf, outb, x_sem, wa_sem, woa_sem, wob_sem, st_sem, out_sem):

    b_weights = (wq_hbm, wk_hbm, wv_hbm)

    def x_copy(r):
        rows = pl.ds(r * XB // 2, XB // 2)
        return pltpu.make_async_copy(x_hbm.bitcast(U32).at[rows], xs.at[rows], x_sem.at[r])

    def wa_copies(n):
        return [pltpu.make_async_copy(
            wa_hbm.bitcast(U32).at[:, _rows(t * 128, 128)], wt.at[WA0 + t], wa_sem.at[n])
            for t in (2 * n, 2 * n + 1)]

    def woa_copy(n):
        return pltpu.make_async_copy(
            woa_hbm.bitcast(U32).at[:, _rows(n * CW, CW)], woa.at[n], woa_sem.at[n])

    def wob_copy(n):
        rows = _rows(n * (HB * DB // 2 // NCG), HB * DB // 2 // NCG)
        return pltpu.make_async_copy(wob_hbm.bitcast(U32).at[rows], wob.at[rows], wob_sem.at[n])

    def stage_copy(part, n):
        rows = _rows(n * WCH, WCH)
        return pltpu.make_async_copy(
            b_weights[part].bitcast(U32).at[rows], stage.at[part, rows], st_sem.at[part * NCG + n])

    def out_copy(qtile, cg):
        rows = _rows(qtile * QT, QT)
        return pltpu.make_async_copy(
            outb.at[cg, rows], out_hbm.at[rows, _rows(cg * CW, CW)], out_sem)

    for cp in wa_copies(0) + [x_copy(0), x_copy(1)]:
        cp.start()

    for i in range(RING - LAG, RING):
        sbuf[i][...] = jnp.zeros((S, QT), F32)
    mcar[...] = jnp.zeros(mcar.shape, F32)
    ot[...] = jnp.zeros(ot.shape, F32)
    oa[1] = jnp.zeros(oa.shape[1:], U32)
    bbuf[1] = jnp.zeros(bbuf.shape[1:], F32)
    gbuf[0:QT, :] = jnp.zeros((QT, 128), F32)
    zero[0] = 0
    gw = jnp.broadcast_to(gw_ref[...].astype(F32).reshape(1, D), (8, D))

    def load_segment(seg):
        xr = _bf(xs[_rows(seg * (SEG // 2), SEG // 2), :]).astype(F32)
        hbuf[MEM:L, :] = xr
        z = jnp.sum(xr.reshape(SEG // 8, 8, D) * gw, axis=-1, keepdims=True).reshape(SEG, 1)
        gbuf[_rows(QT + seg * SEG, SEG), :] = jnp.broadcast_to(
            1.0 / (1.0 + jnp.exp(-z)), (SEG, 128))

    def relayout(part, group, halves=(0, 1)):
        w = stage[part, _rows(group * 16 * HB // 2, 16 * HB // 2), :].reshape(8, 2, HB // 2, 128)
        rows = _rows(group * 8, 8)
        for half in halves:
            a, b = w[:, 0, half * 8:(half + 1) * 8], w[:, 1, half * 8:(half + 1) * 8]
            lo = (a & U32(0xFFFF)) | (b << 16)
            hi = (a >> 16) | (b & U32(0xFFFF0000))
            for odd, t in enumerate((lo, hi)):
                v = _transpose8([t[i] for i in range(8)])
                for j in range(8):
                    wt[3 * (2 * (half * 8 + j) + odd) + part, rows, :] = v[j]

    def project(part, tile, m):
        rows = _rows(m * (MC // 2), MC // 2)
        y = _dot(_bf(xs[rows, :]), _bf(wt[WA0 + part * (D // 128) + tile]))
        if part == 2:
            col = (m * MC) % KC
            vt[(m * MC) // KC, pl.ds(tile * (128 // DA), 128 // DA), :, col:col + MC] = (
                _words(y.T).reshape(128 // DA, DA // 2, MC))
        elif part == 1:
            ka[tile, rows, :] = _words(y)
        else:
            qa[tile, rows, :] = _words(y * (DA ** -0.5 * LOG2E))

    waits = [[x_copy(r)] for r in range(NX)] + [wa_copies(1)]
    waits[0] += wa_copies(0)
    starts = [[x_copy(2)], [x_copy(3)], wa_copies(1), [stage_copy(0, 0)],
              wa_copies(2) + [stage_copy(0, 1)] + wa_copies(3)]

    def first_body(i, carry):
        for k, (ws, ss) in enumerate(zip(waits, starts)):
            @pl.when(i == k)
            def _(ws=ws, ss=ss):
                for cp in ws:
                    cp.wait()
                for cp in ss:
                    cp.start()

        for m in range(XB // MC):
            for t in range(2):
                project(0, 2 * (i // NX) + t, (i % NX) * (XB // MC) + m)
        return carry

    jax.lax.fori_loop(0, 2 * NX, first_body, 0)
    hbuf[0:MEM, :] = mem_ref[...].astype(F32)
    load_segment(0)

    for part in range(3):
        def proj_body(n, carry, part=part):
            cur = part * NCG + n
            chunk = n - 2 if part == 0 else n
            for cp in wa_copies(cur):
                cp.wait()
            stage_copy(part, chunk).wait()

            @pl.when(cur + 2 < 3 * NCG)
            def _():
                for cp in wa_copies(cur + 2):
                    cp.start()

            if part == 0:
                stage_copy(1, chunk).start()
            else:
                @pl.when(n + 2 < NCG)
                def _():
                    stage_copy(part, n + 2).start()

            if part == 1:
                @pl.when(n + 2 >= NCG)
                def _():
                    stage_copy(2, n + 2 - NCG).start()

                wob_copy(n).start()
            if part == 2:
                woa_copy(n).start()

            for g in range(16):
                project(part, 2 * n + g % 2, g // 2)
                relayout(part, chunk * 16 + g)
                if part > 0 and g % 2 == 0:
                    relayout(0, (1 + part) * 16 + 4 * n + g // 4, halves=(g // 2 % 2,))
            return carry

        if part < 2:
            stage_copy(0, 2 + part).start()
        if part > 0:
            stage_copy(0, 1 + part).wait()
        jax.lax.fori_loop(2 if part == 0 else 0, NCG, proj_body, 0)

    for n in range(NCG):
        woa_copy(n).wait()
        wob_copy(n).wait()

    row = jax.lax.broadcasted_iota(jnp.int32, (L, L), 0)
    col = jax.lax.broadcasted_iota(jnp.int32, (L, L), 1)
    mask_b = (row < MEM) | (row >= col)
    head_lane = jax.lax.broadcasted_iota(jnp.int32, (QT // 2, 128), 1) // DA

    def a_scores(tile, qtile, i, c):
        q = qa[tile, _rows(qtile * (QT // 2), QT // 2), :]
        q = _bf(jnp.where(head_lane == i % 4, q, U32(0)))
        mx = None
        n = KC // 4
        for r in range(c * KC, (c + 1) * KC, n):
            st = _dot_nt(_bf(ka[tile, r // 2:(r + n) // 2, :]), q)
            sbuf[i % RING][r:r + n, :] = st
            m = st.reshape(n // 8, 8, 128).max(axis=0)
            mx = m if mx is None else jnp.maximum(mx, m)
        return mx

    def not_before(x, other):
        nop = pltpu.bitcast(other[0:8, 0:QT], U32) & zero[0].astype(U32)
        return pltpu.bitcast(pltpu.bitcast(x, U32) | nop, F32)

    def a_probs(i, c, m):
        st = sbuf[i % RING][_rows(zero[0] + c * KC, KC), :].reshape(KC // 8, 8, QT)
        p = jnp.exp2(st - m).reshape(KC, QT)
        return p.astype(BF16), p.reshape(KC // 32, 32, QT).sum(axis=0)

    def a_values(head, c, p):
        return _dot(_bf(vt[c, head]), p)

    def a_finish(i, acc, den):
        ot[i * DA:(i + 1) * DA, :] = acc * _recip(jnp.sum(den, axis=0, keepdims=True))

    def a_transpose(qtile, tile, which):
        oa[qtile % 2, tile] = _words(ot[which * 128:(which + 1) * 128, :].T)

    def mix(qtile, cg):
        o = jnp.concatenate([_bf(oa[qtile % 2, t]) for t in range(D // 128)], axis=1)
        a = _dot(o, _bf(woa[cg]))
        g = gbuf[_rows((qtile + 1) * QT, QT), :]
        g = jnp.concatenate([g] * (CW // 128), axis=1)
        outb[cg, _rows(jnp.maximum(qtile, 0) * QT, QT), :] = (
            g * a + (1.0 - g) * bbuf[qtile % 2, cg]).astype(BF16)

    def b_project(tile):
        return _dot(hbuf[...], _bf(wt[tile]))

    def b_scores(q, k):
        sc = jnp.where(mask_b, _dot_nt(q, k), -1e9 * LOG2E)
        pr = jnp.exp2(sc - jnp.max(sc, axis=-1, keepdims=True))
        return pr * _recip(jnp.sum(pr, axis=-1, keepdims=True))

    def b_values(head, pr, v):
        obuf[:, head * DB:(head + 1) * DB] = _dot(pr, v)

    def b_out(h0, h1):
        return _dot(obuf[:, h0 * DB:h1 * DB], _bf(wob[h0 * DB // 2:h1 * DB // 2, :]))

    def step(s, ends_loop_body):
        qtile, cg = s // NCG, s % NCG
        cg_prev = (s + NCG - 1) % NCG
        maxes = {i - LAG: mcar[i] for i in range(LAG)}
        probs, values = {}, {}
        for h in range(HB):
            i, c = h // NC, h % NC
            ip = i - LAG
            if h >= 1:
                probs[h - 1] = b_scores(q, k)
            y = b_project(3 * h)
            q = y * (DB ** -0.5 * LOG2E)
            p, den = a_probs(ip, c, not_before(maxes[ip], y))
            dsum = den if c == 0 else dsum + den
            k = b_project(3 * h + 1).astype(BF16)
            mx = a_scores(2 * cg + i // 4, qtile, i, c)
            m_run = mx if c == 0 else jnp.maximum(m_run, mx)
            values[h] = b_project(3 * h + 2).astype(BF16)
            o = a_values(NI * cg + ip if ip >= 0 else NI * cg_prev + NI + ip, c, p)
            acc = o if c == 0 else acc + o
            if h >= 3:
                b_values(h - 3, probs.pop(h - 3), values.pop(h - 3))
            if c == NC - 1:
                a_finish(ip % NI, acc, dsum)
                maxes[i] = jnp.broadcast_to(jnp.max(m_run, axis=0, keepdims=True), (8, QT))
            if h == LAG * NC + 1:
                a_transpose((s + 2 * NCG - 1) // NCG, 2 * cg_prev + 1, 1)
            if h == (LAG + 4) * NC + 1:
                a_transpose(qtile, 2 * cg, 0)
        for i in range(LAG):
            mcar[i] = maxes[NI - LAG + i]

        nxt = jnp.minimum(s + 1, NSTEP - 1)
        if not ends_loop_body:
            load_segment(nxt)
        cut = 11 if ends_loop_body else 13
        y = b_out(0, 2)
        probs[HB - 1] = b_scores(q, k)
        b_values(HB - 3, probs[HB - 3], values[HB - 3])
        y = y + b_out(2, 6)
        b_values(HB - 2, probs[HB - 2], values[HB - 2])
        y = y + b_out(6, cut)
        b_values(HB - 1, probs[HB - 1], values[HB - 1])
        if ends_loop_body:
            y = y + b_out(cut, 14)
            load_segment(nxt)
            y = y + b_out(14, 26)
            mix(qtile - 1, cg)
            y = y + b_out(26, HB)
        else:
            y = y + b_out(cut, HB)
            mix(qtile - 1, cg)
        hbuf[0:MEM, :] = y[0:MEM].astype(BF16).astype(F32)
        for t in range(NCG):
            bbuf[qtile % 2, t, _rows(cg * SEG, SEG), :] = y[MEM:L, t * CW:(t + 1) * CW]

    def two_steps(t, carry):
        step(2 * t, False)
        step(2 * t + 1, True)

        @pl.when(t >= NCG // 2)
        def _():
            for u in range(2):
                out_copy((2 * t) // NCG - 1, (2 * t) % NCG + u).start()
        return carry

    jax.lax.fori_loop(0, NSTEP // 2, two_steps, 0)

    for i in range(LAG):
        for c in range(NC):
            p, den = a_probs(i - LAG, c, mcar[i])
            o = a_values(HA - LAG + i, c, p)
            acc, dsum = (o, den) if c == 0 else (acc + o, dsum + den)
        a_finish(NI - LAG + i, acc, dsum)
    last = S // QT - 1
    a_transpose(last, D // 128 - 1, 1)
    for cg in range(NCG):
        mix(last, cg)
        out_copy(last, cg).start()

    def wait_body(t, carry):
        out_copy(t // NCG, t % NCG).wait()
        return carry

    jax.lax.fori_loop(0, (S // QT) * NCG, wait_body, 0)


@jax.jit
def pallas_gated_mix__softmax_full_mha__memory_aug_recurrent_mem_tr__prompt_kernel(
    A_x: jax.Array,
    A_wqkv: jax.Array,
    A_wo: jax.Array,
    B_x: jax.Array,
    B_mem0: jax.Array,
    B_Wq: jax.Array,
    B_Wk: jax.Array,
    B_Wv: jax.Array,
    B_Wo: jax.Array,
    B_seg_len: jax.Array,
    gate_w: jax.Array,
):
    del B_x, B_seg_len
    assert A_x.shape == (1, S, D) and B_mem0.shape == (1, MEM, D) and B_Wq.shape == (D, HB, DB)

    hbm = pl.BlockSpec(memory_space=pl.ANY)
    vmem = pl.BlockSpec(memory_space=pltpu.VMEM)
    out = pl.pallas_call(
        _kernel,
        out_shape=jax.ShapeDtypeStruct((S, D), BF16),
        in_specs=[hbm, hbm, hbm, vmem, hbm, hbm, hbm, hbm, vmem],
        out_specs=hbm,
        scratch_shapes=[
            pltpu.VMEM((S // 2, D), U32),
            pltpu.VMEM((WA0 + 3 * D // 128, D // 2, 128), U32),
            pltpu.VMEM((NCG, D // 2, CW), U32),
            pltpu.VMEM((HB * DB // 2, D), U32),
            pltpu.VMEM((3, D * HB // 2, DB), U32),
            pltpu.VMEM((D // 128, S // 2, 128), U32),
            pltpu.VMEM((D // 128, S // 2, 128), U32),
            pltpu.VMEM((NC, HA, DA // 2, KC), U32),
            [pltpu.VMEM((S, QT), F32)] * RING,
            pltpu.SMEM((1,), jnp.int32),
            pltpu.VMEM((LAG, 8, QT), F32),
            pltpu.VMEM((NI * DA, QT), F32),
            pltpu.VMEM((2, D // 128, QT // 2, 128), U32),
            pltpu.VMEM((L, D), F32),
            pltpu.VMEM((L, HB * DB), F32),
            pltpu.VMEM((2, NCG, QT, CW), F32),
            pltpu.VMEM((QT + S, 128), F32),
            pltpu.VMEM((NCG, S, CW), BF16),
            pltpu.SemaphoreType.DMA((NX,)),
            pltpu.SemaphoreType.DMA((3 * NCG,)),
            pltpu.SemaphoreType.DMA((NCG,)),
            pltpu.SemaphoreType.DMA((NCG,)),
            pltpu.SemaphoreType.DMA((3 * NCG,)),
            pltpu.SemaphoreType.DMA(()),
        ],
        compiler_params=pltpu.CompilerParams(vmem_limit_bytes=110 * 1024 * 1024),
        name="gated_mix",
    )(
        A_x.reshape(S, D), A_wqkv, A_wo, B_mem0.reshape(MEM, D),
        B_Wq.reshape(D * HB, DB), B_Wk.reshape(D * HB, DB), B_Wv.reshape(D * HB, DB),
        B_Wo.reshape(HB * DB, D), gate_w,
    )
    return out.reshape(1, S, D)
```

```python
import math

import jax
import jax.numpy as jnp
import jax.experimental.pallas as pl
import jax.experimental.pallas.tpu as pltpu

BF16, F32, U32 = jnp.bfloat16, jnp.float32, jnp.uint32
LOG2E = math.log2(math.e)

S, D = 2048, 1024
HA, DA = 32, 32
HB, DB = 32, 128
MEM, SEG = 8, 32
L = MEM + SEG
NSTEP = S // SEG
QT = 128
KC = 512
NC = S // KC
NI = HB // NC
LAG = 2
RING = 4
CW = 256
NCG = D // CW
MC = 256
XB = 512
NX = S // XB
WA0 = 3 * HB
WCH = D * HB // 2 // NCG


def _bf(x):
    return pltpu.bitcast(x, BF16)


def _words(x):
    return pltpu.bitcast(x.astype(BF16), U32)


def _dot(a, b):
    return jnp.dot(a, b, preferred_element_type=F32)


def _dot_nt(a, b):
    return jax.lax.dot_general(a, b, (((1,), (1,)), ((), ())), preferred_element_type=F32)


def _recip(x):
    r = pltpu.reciprocal(x, approx=True)
    return r * (2.0 - x * r)


def _rows(start, n):
    return pl.ds(pl.multiple_of(start, n), n)


def _transpose8(v):
    sub = jax.lax.broadcasted_iota(U32, (8, 128), 0)
    for s in (4, 2, 1):
        keep = (sub & s) == 0
        nv = list(v)
        for i in range(8):
            if i & s == 0:
                a, b = v[i], v[i + s]
                nv[i] = jnp.where(keep, a, pltpu.roll(b, s, 0))
                nv[i + s] = jnp.where(keep, pltpu.roll(a, 8 - s, 0), b)
        v = nv
    return v


def _kernel(x_hbm, wa_hbm, woa_hbm, mem_ref, wq_hbm, wk_hbm, wv_hbm, wob_hbm, gw_ref, out_hbm,
            xs, wt, woa, wob, stage, ka, qa, vt, sbuf, zero, mcar, ot, oa,
            hbuf, obuf, bbuf, gbuf, outb, x_sem, wa_sem, woa_sem, wob_sem, st_sem, out_sem):

    b_weights = (wq_hbm, wk_hbm, wv_hbm)

    def x_copy(r):
        rows = pl.ds(r * XB // 2, XB // 2)
        return pltpu.make_async_copy(x_hbm.bitcast(U32).at[rows], xs.at[rows], x_sem.at[r])

    def wa_copies(n):
        return [pltpu.make_async_copy(
            wa_hbm.bitcast(U32).at[:, _rows(t * 128, 128)], wt.at[WA0 + t], wa_sem.at[n])
            for t in (2 * n, 2 * n + 1)]

    def woa_copy(n):
        return pltpu.make_async_copy(
            woa_hbm.bitcast(U32).at[:, _rows(n * CW, CW)], woa.at[n], woa_sem.at[n])

    def wob_copy(n):
        rows = _rows(n * (HB * DB // 2 // NCG), HB * DB // 2 // NCG)
        return pltpu.make_async_copy(wob_hbm.bitcast(U32).at[rows], wob.at[rows], wob_sem.at[n])

    def stage_copy(part, n):
        rows = _rows(n * WCH, WCH)
        return pltpu.make_async_copy(
            b_weights[part].bitcast(U32).at[rows], stage.at[part, rows], st_sem.at[part * NCG + n])

    def out_copy(qtile, cg):
        rows = _rows(qtile * QT, QT)
        return pltpu.make_async_copy(
            outb.at[cg, rows], out_hbm.at[rows, _rows(cg * CW, CW)], out_sem)

    for cp in wa_copies(0) + [x_copy(0), x_copy(1)]:
        cp.start()

    for i in range(RING - LAG, RING):
        sbuf[i][...] = jnp.zeros((S, QT), F32)
    mcar[...] = jnp.zeros(mcar.shape, F32)
    ot[...] = jnp.zeros(ot.shape, F32)
    oa[1] = jnp.zeros(oa.shape[1:], U32)
    bbuf[1] = jnp.zeros(bbuf.shape[1:], F32)
    gbuf[0:QT, :] = jnp.zeros((QT, 128), F32)
    zero[0] = 0
    gw = jnp.broadcast_to(gw_ref[...].astype(F32).reshape(1, D), (8, D))

    def load_segment(seg):
        xr = _bf(xs[_rows(seg * (SEG // 2), SEG // 2), :]).astype(F32)
        hbuf[MEM:L, :] = xr
        z = jnp.sum(xr.reshape(SEG // 8, 8, D) * gw, axis=-1, keepdims=True).reshape(SEG, 1)
        gbuf[_rows(QT + seg * SEG, SEG), :] = jnp.broadcast_to(
            1.0 / (1.0 + jnp.exp(-z)), (SEG, 128))

    def relayout(part, group, quarters=range(4)):
        w = stage[part, _rows(group * 16 * HB // 2, 16 * HB // 2), :].reshape(8, 2, HB // 2, 128)
        rows = _rows(group * 8, 8)
        for quarter in quarters:
            half, odd = quarter // 2, quarter % 2
            a, b = w[:, 0, half * 8:(half + 1) * 8], w[:, 1, half * 8:(half + 1) * 8]
            if odd:
                t = (a >> 16) | (b & U32(0xFFFF0000))
            else:
                t = (a & U32(0xFFFF)) | (b << 16)
            v = _transpose8([t[i] for i in range(8)])
            for j in range(8):
                wt[3 * (2 * (half * 8 + j) + odd) + part, rows, :] = v[j]

    def project(part, tile, m):
        rows = _rows(m * (MC // 2), MC // 2)
        y = _dot(_bf(xs[rows, :]), _bf(wt[WA0 + part * (D // 128) + tile]))
        if part == 2:
            col = (m * MC) % KC
            vt[(m * MC) // KC, pl.ds(tile * (128 // DA), 128 // DA), :, col:col + MC] = (
                _words(y.T).reshape(128 // DA, DA // 2, MC))
        elif part == 1:
            ka[tile, rows, :] = _words(y)
        else:
            qa[tile, rows, :] = _words(y * (DA ** -0.5 * LOG2E))

    waits = [[x_copy(r)] for r in range(NX)] + [wa_copies(1)]
    waits[0] += wa_copies(0)
    starts = [[x_copy(2)], [x_copy(3)], wa_copies(1), [stage_copy(0, 0)],
              wa_copies(2) + [stage_copy(0, 1)] + wa_copies(3)]

    def first_body(i, carry):
        for k, (ws, ss) in enumerate(zip(waits, starts)):
            @pl.when(i == k)
            def _(ws=ws, ss=ss):
                for cp in ws:
                    cp.wait()
                for cp in ss:
                    cp.start()

        for m in range(XB // MC):
            for t in range(2):
                project(0, 2 * (i // NX) + t, (i % NX) * (XB // MC) + m)
        return carry

    jax.lax.fori_loop(0, 2 * NX, first_body, 0)
    hbuf[0:MEM, :] = mem_ref[...].astype(F32)
    load_segment(0)

    for part in range(3):
        def proj_body(n, carry, part=part):
            cur = part * NCG + n
            chunk = n - 2 if part == 0 else n
            for cp in wa_copies(cur):
                cp.wait()
            stage_copy(part, chunk).wait()

            @pl.when(cur + 2 < 3 * NCG)
            def _():
                for cp in wa_copies(cur + 2):
                    cp.start()

            if part == 0:
                stage_copy(1, chunk).start()
            else:
                @pl.when(n + 2 < NCG)
                def _():
                    stage_copy(part, n + 2).start()

            if part == 1:
                @pl.when(n + 2 >= NCG)
                def _():
                    stage_copy(2, n + 2 - NCG).start()

                wob_copy(n).start()
            if part == 2:
                woa_copy(n).start()

            for g in range(16):
                project(part, 2 * n + g % 2, g // 2)
                relayout(part, chunk * 16 + g)
                if part > 0:
                    relayout(0, (1 + part) * 16 + 4 * n + g // 4, quarters=(g % 4,))
            return carry

        if part < 2:
            stage_copy(0, 2 + part).start()
        if part > 0:
            stage_copy(0, 1 + part).wait()
        jax.lax.fori_loop(2 if part == 0 else 0, NCG, proj_body, 0)

    for n in range(NCG):
        woa_copy(n).wait()
        wob_copy(n).wait()

    row = jax.lax.broadcasted_iota(jnp.int32, (L, L), 0)
    col = jax.lax.broadcasted_iota(jnp.int32, (L, L), 1)
    mask_b = (row < MEM) | (row >= col)
    head_lane = jax.lax.broadcasted_iota(jnp.int32, (QT // 2, 128), 1) // DA

    def a_scores(tile, qtile, i, c):
        q = qa[tile, _rows(qtile * (QT // 2), QT // 2), :]
        q = _bf(jnp.where(head_lane == i % 4, q, U32(0)))
        mx = None
        n = KC // 4
        for r in range(c * KC, (c + 1) * KC, n):
            st = _dot_nt(_bf(ka[tile, r // 2:(r + n) // 2, :]), q)
            sbuf[i % RING][r:r + n, :] = st
            m = st.reshape(n // 8, 8, 128).max(axis=0)
            mx = m if mx is None else jnp.maximum(mx, m)
        return mx

    def not_before(x, other):
        nop = pltpu.bitcast(other[0:8, 0:QT], U32) & zero[0].astype(U32)
        return pltpu.bitcast(pltpu.bitcast(x, U32) | nop, F32)

    def a_probs(i, c, m):
        st = sbuf[i % RING][_rows(zero[0] + c * KC, KC), :].reshape(KC // 8, 8, QT)
        p = jnp.exp2(st - m).reshape(KC, QT)
        return p.astype(BF16), p.reshape(KC // 32, 32, QT).sum(axis=0)

    def a_values(head, c, p):
        return _dot(_bf(vt[c, head]), p)

    def a_finish(i, acc, den):
        ot[i * DA:(i + 1) * DA, :] = acc * _recip(jnp.sum(den, axis=0, keepdims=True))

    def a_transpose(qtile, tile, which):
        oa[qtile % 2, tile] = _words(ot[which * 128:(which + 1) * 128, :].T)

    def mix(qtile, cg):
        o = jnp.concatenate([_bf(oa[qtile % 2, t]) for t in range(D // 128)], axis=1)
        a = _dot(o, _bf(woa[cg]))
        g = gbuf[_rows((qtile + 1) * QT, QT), :]
        g = jnp.concatenate([g] * (CW // 128), axis=1)
        outb[cg, _rows(jnp.maximum(qtile, 0) * QT, QT), :] = (
            g * a + (1.0 - g) * bbuf[qtile % 2, cg]).astype(BF16)

    def b_project(tile):
        return _dot(hbuf[...], _bf(wt[tile]))

    def b_scores(q, k):
        sc = jnp.where(mask_b, _dot_nt(q, k), -1e9 * LOG2E)
        pr = jnp.exp2(sc - jnp.max(sc, axis=-1, keepdims=True))
        return pr * _recip(jnp.sum(pr, axis=-1, keepdims=True))

    def b_values(head, pr, v):
        obuf[:, head * DB:(head + 1) * DB] = _dot(pr, v)

    def b_out(h0, h1):
        return _dot(obuf[:, h0 * DB:h1 * DB], _bf(wob[h0 * DB // 2:h1 * DB // 2, :]))

    def step(s, ends_loop_body):
        qtile, cg = s // NCG, s % NCG
        cg_prev = (s + NCG - 1) % NCG
        maxes = {i - LAG: mcar[i] for i in range(LAG)}
        probs, values = {}, {}
        for h in range(HB):
            i, c = h // NC, h % NC
            ip = i - LAG
            if h >= 1:
                probs[h - 1] = b_scores(q, k)
            y = b_project(3 * h)
            q = y * (DB ** -0.5 * LOG2E)
            p, den = a_probs(ip, c, not_before(maxes[ip], y))
            dsum = den if c == 0 else dsum + den
            k = b_project(3 * h + 1).astype(BF16)
            mx = a_scores(2 * cg + i // 4, qtile, i, c)
            m_run = mx if c == 0 else jnp.maximum(m_run, mx)
            values[h] = b_project(3 * h + 2).astype(BF16)
            o = a_values(NI * cg + ip if ip >= 0 else NI * cg_prev + NI + ip, c, p)
            acc = o if c == 0 else acc + o
            if h >= 3:
                b_values(h - 3, probs.pop(h - 3), values.pop(h - 3))
            if c == NC - 1:
                a_finish(ip % NI, acc, dsum)
                maxes[i] = jnp.broadcast_to(jnp.max(m_run, axis=0, keepdims=True), (8, QT))
            if h == LAG * NC + 1:
                a_transpose((s + 2 * NCG - 1) // NCG, 2 * cg_prev + 1, 1)
            if h == (LAG + 4) * NC + 1:
                a_transpose(qtile, 2 * cg, 0)
        for i in range(LAG):
            mcar[i] = maxes[NI - LAG + i]

        nxt = jnp.minimum(s + 1, NSTEP - 1)
        if not ends_loop_body:
            load_segment(nxt)
        cut = 11 if ends_loop_body else 13
        y = b_out(0, 2)
        probs[HB - 1] = b_scores(q, k)
        b_values(HB - 3, probs[HB - 3], values[HB - 3])
        y = y + b_out(2, 6)
        b_values(HB - 2, probs[HB - 2], values[HB - 2])
        y = y + b_out(6, cut)
        b_values(HB - 1, probs[HB - 1], values[HB - 1])
        if ends_loop_body:
            y = y + b_out(cut, 14)
            load_segment(nxt)
            y = y + b_out(14, 26)
            mix(qtile - 1, cg)
            y = y + b_out(26, HB)
        else:
            y = y + b_out(cut, HB)
            mix(qtile - 1, cg)
        hbuf[0:MEM, :] = y[0:MEM].astype(BF16).astype(F32)
        for t in range(NCG):
            bbuf[qtile % 2, t, _rows(cg * SEG, SEG), :] = y[MEM:L, t * CW:(t + 1) * CW]

    def two_steps(t, carry):
        step(2 * t, False)
        step(2 * t + 1, True)

        @pl.when(t >= NCG // 2)
        def _():
            for u in range(2):
                out_copy((2 * t) // NCG - 1, (2 * t) % NCG + u).start()
        return carry

    jax.lax.fori_loop(0, NSTEP // 2, two_steps, 0)

    for i in range(LAG):
        for c in range(NC):
            p, den = a_probs(i - LAG, c, mcar[i])
            o = a_values(HA - LAG + i, c, p)
            acc, dsum = (o, den) if c == 0 else (acc + o, dsum + den)
        a_finish(NI - LAG + i, acc, dsum)
    last = S // QT - 1
    a_transpose(last, D // 128 - 1, 1)
    for cg in range(NCG):
        mix(last, cg)
        out_copy(last, cg).start()

    def wait_body(t, carry):
        out_copy(t // NCG, t % NCG).wait()
        return carry

    jax.lax.fori_loop(0, (S // QT) * NCG, wait_body, 0)


@jax.jit
def pallas_gated_mix__softmax_full_mha__memory_aug_recurrent_mem_tr__prompt_kernel(
    A_x: jax.Array,
    A_wqkv: jax.Array,
    A_wo: jax.Array,
    B_x: jax.Array,
    B_mem0: jax.Array,
    B_Wq: jax.Array,
    B_Wk: jax.Array,
    B_Wv: jax.Array,
    B_Wo: jax.Array,
    B_seg_len: jax.Array,
    gate_w: jax.Array,
):
    del B_x, B_seg_len
    assert A_x.shape == (1, S, D) and B_mem0.shape == (1, MEM, D) and B_Wq.shape == (D, HB, DB)

    hbm = pl.BlockSpec(memory_space=pl.ANY)
    vmem = pl.BlockSpec(memory_space=pltpu.VMEM)
    out = pl.pallas_call(
        _kernel,
        out_shape=jax.ShapeDtypeStruct((S, D), BF16),
        in_specs=[hbm, hbm, hbm, vmem, hbm, hbm, hbm, hbm, vmem],
        out_specs=hbm,
        scratch_shapes=[
            pltpu.VMEM((S // 2, D), U32),
            pltpu.VMEM((WA0 + 3 * D // 128, D // 2, 128), U32),
            pltpu.VMEM((NCG, D // 2, CW), U32),
            pltpu.VMEM((HB * DB // 2, D), U32),
            pltpu.VMEM((3, D * HB // 2, DB), U32),
            pltpu.VMEM((D // 128, S // 2, 128), U32),
            pltpu.VMEM((D // 128, S // 2, 128), U32),
            pltpu.VMEM((NC, HA, DA // 2, KC), U32),
            [pltpu.VMEM((S, QT), F32)] * RING,
            pltpu.SMEM((1,), jnp.int32),
            pltpu.VMEM((LAG, 8, QT), F32),
            pltpu.VMEM((NI * DA, QT), F32),
            pltpu.VMEM((2, D // 128, QT // 2, 128), U32),
            pltpu.VMEM((L, D), F32),
            pltpu.VMEM((L, HB * DB), F32),
            pltpu.VMEM((2, NCG, QT, CW), F32),
            pltpu.VMEM((QT + S, 128), F32),
            pltpu.VMEM((NCG, S, CW), BF16),
            pltpu.SemaphoreType.DMA((NX,)),
            pltpu.SemaphoreType.DMA((3 * NCG,)),
            pltpu.SemaphoreType.DMA((NCG,)),
            pltpu.SemaphoreType.DMA((NCG,)),
            pltpu.SemaphoreType.DMA((3 * NCG,)),
            pltpu.SemaphoreType.DMA(()),
        ],
        compiler_params=pltpu.CompilerParams(vmem_limit_bytes=110 * 1024 * 1024),
        name="gated_mix",
    )(
        A_x.reshape(S, D), A_wqkv, A_wo, B_mem0.reshape(MEM, D),
        B_Wq.reshape(D * HB, DB), B_Wk.reshape(D * HB, DB), B_Wv.reshape(D * HB, DB),
        B_Wo.reshape(HB * DB, D), gate_w,
    )
    return out.reshape(1, S, D)
```
